```python
import jax
import jax.numpy as jnp

def _softmax(x, axis=-1):
    return jax.nn.softmax(x, axis=axis)
def _gelu(x):
    return jax.nn.gelu(x, approximate=True)
def _silu(x):
    return jax.nn.silu(x)
def _sigmoid(x):
    return jax.nn.sigmoid(x)
def _layernorm(x, axis=-1, eps=1e-5):
    m = jnp.mean(x, axis=axis, keepdims=True)
    v = jnp.var(x, axis=axis, keepdims=True)
    return (x - m) / jnp.sqrt(v + eps)
def _scatter_add(tgt, idx, src, axis=0):
    return tgt.at[idx].add(src)
def _segment_sum(src, seg, n):
    return jax.ops.segment_sum(src, seg, n)
class _Rng:
    def __init__(self, key):
        self._k = key
    def _next(self):
        self._k, sub = jax.random.split(self._k)
        return sub
    def normal(self, shape):
        return jax.random.normal(self._next(), shape, dtype=jnp.bfloat16)
    def randint(self, lo, hi, shape):
        return jax.random.randint(self._next(), shape, lo, hi, dtype=jnp.int32)
    def uniform(self, shape, lo=0.0, hi=1.0):
        return jax.random.uniform(self._next(), shape, jnp.bfloat16, lo, hi)
    def permutation(self, n):
        return jax.random.permutation(self._next(), n)


kernel_name = 'concat_heads__ssm_conv_h3__compressed_kv_cla__prompt'

def setup_inputs():
    _rng = _Rng(jax.random.key(int.from_bytes(__import__("os").urandom(4), "little")))
    _w = (lambda a: (lambda t: t.astype(jnp.bfloat16) if jnp.issubdtype(t.dtype, jnp.floating) else t)(jnp.asarray(a)))
    def _A_setup():
        B, S, D = 1, 2048, 448
        ks = 4
        return {
            "q": _w((lambda *s: _rng.normal(s) * 0.05)(B, S, D)),
            "k": _w((lambda *s: _rng.normal(s) * 0.05)(B, S, D)),
            "v": _w((lambda *s: _rng.normal(s) * 0.05)(B, S, D)),
            "shift_k": _w((lambda *s: _rng.normal(s) * 0.05)(D, ks) * 0.5),
            "ssm_k": _w((lambda *s: _rng.normal(s) * 0.05)(D, S) * (1.0 / S ** 0.5)),
            "ssm_D": _w((lambda *s: _rng.normal(s) * 0.05)(D)),
        }
    _A_in = _A_setup()

    def _B_setup():
        B, H, Sq, Sk, D, M = 1, 16, 2048, 2048, 256, 448
        Dc = 4 * D
        return {
            "x": _w((lambda *s: _rng.normal(s) * 0.05)(B, Sq, M)),
            "c_kv": _w((lambda *s: _rng.normal(s) * 0.05)(B, Sk, Dc)),
            "w_q": _w((lambda *s: _rng.normal(s) * 0.05)(M, H, D) * (M ** -0.5)),
            "w_uk": _w((lambda *s: _rng.normal(s) * 0.05)(Dc, H, D) * (Dc ** -0.5)),
            "w_uv": _w((lambda *s: _rng.normal(s) * 0.05)(Dc, H, D) * (Dc ** -0.5)),
            "w_o": _w((lambda *s: _rng.normal(s) * 0.05)(H, D, M) * ((H * D) ** -0.5)),
        }
    _B_in = _B_setup()

    return {
        "A_q": _A_in["q"],
        "A_k": _A_in["k"],
        "A_v": _A_in["v"],
        "A_shift_k": _A_in["shift_k"],
        "A_ssm_k": _A_in["ssm_k"],
        "A_ssm_D": _A_in["ssm_D"],
        "B_x": _B_in["x"],
        "B_c_kv": _B_in["c_kv"],
        "B_w_q": _B_in["w_q"],
        "B_w_uk": _B_in["w_uk"],
        "B_w_uv": _B_in["w_uv"],
        "B_w_o": _B_in["w_o"],
    }

def reference(A_q, A_k, A_v, A_shift_k, A_ssm_k, A_ssm_D, B_x, B_c_kv, B_w_q, B_w_uk, B_w_uv, B_w_o):
    def _A_ref(q, k, v, shift_k, ssm_k, ssm_D):
        B, S, D = q.shape
        ks = shift_k.shape[-1]
        k_pad = jnp.pad(k, ((0, 0), (ks - 1, 0), (0, 0)))
        k_shift = jnp.zeros_like(k)
        for t in range(ks):
            k_shift = k_shift + k_pad[:, t:t + S, :] * shift_k[:, ks - 1 - t][None, None, :]
        kv = k_shift * v
        L = 2 * S
        kv_pad = jnp.pad(kv, ((0, 0), (0, S), (0, 0)))
        kf_pad = jnp.pad(ssm_k, ((0, 0), (0, S)))
        kv_f = (lambda x, axes=(-2,-1): jnp.fft.rfft2(x.astype(jnp.float32), axes=axes))(kv_pad[:, None, :, :], axes=(1, 2))
        kf_f = (lambda x, axes=(-2,-1): jnp.fft.rfft2(x.astype(jnp.float32), axes=axes))(kf_pad[:, None, :], axes=(1, 2))
        kf_f = (lambda x, *d: x.transpose(*d))(kf_f, 1, 2, 0)
        y_f = kv_f * kf_f[None, :, :, :]
        y = (lambda x, s, axes=(-2,-1): jnp.fft.irfft2(x, s=s, axes=axes).astype(jnp.bfloat16))(y_f, (1, L), axes=(1, 2))[:, 0, :S, :]
        y = y + kv * ssm_D[None, None, :]
        return q * y

    def _B_ref(x, c_kv, w_q, w_uk, w_uv, w_o):
        B, Sq, M = x.shape[0], x.shape[1], x.shape[2]
        Sk = c_kv.shape[1]
        H, D = w_q.shape[1], w_q.shape[2]
        q = jnp.einsum("bqm,mhd->bhqd", x, w_q)
        k = jnp.einsum("bkc,chd->bhkd", c_kv, w_uk)
        v = jnp.einsum("bkc,chd->bhkd", c_kv, w_uv)
        scores = jnp.einsum("bhqd,bhkd->bhqk", q, k) * (D ** -0.5)
        off = Sk - Sq
        qi = jnp.arange(Sq)[:, None]
        kj = jnp.arange(Sk)[None, :]
        cmask = kj <= (qi + off)
        scores = jnp.where(cmask[None, None], scores, -1e9)
        p = _softmax(scores, axis=-1)
        ctx = jnp.einsum("bhqk,bhkd->bhqd", p, v)
        return jnp.einsum("bhqd,hdm->bqm", ctx, w_o)

    a = _A_ref(A_q, A_k, A_v, A_shift_k, A_ssm_k, A_ssm_D)
    b = _B_ref(B_x, B_c_kv, B_w_q, B_w_uk, B_w_uv, B_w_o)
    return jnp.concatenate([a, b], axis=-1)
```

```python
import numpy as np
import jax
import jax.numpy as jnp
from jax import lax
import jax.experimental.pallas as pl
import jax.experimental.pallas.tpu as pltpu

f32 = jnp.float32
bf16 = jnp.bfloat16
NT = (((1,), (1,)), ((), ()))

S = 2048
M = 448
H = 16
D = 256
C = 1024
T = 128
NB = S // T
BQ = 256
CH = 32
NEG = -1e30
QSCALE = float(D ** -0.5 * np.log2(np.e))


def _dft_mats():
    n = np.arange(T)[:, None]
    f = np.arange(T)[None, :]
    th = 2 * np.pi * (f + 0.5) * n / (2 * T)
    fwd = np.concatenate([np.cos(th), -np.sin(th)], axis=1)
    n2 = (T + np.arange(T))[None, :]
    f2 = np.arange(T)[:, None]
    th2 = 2 * np.pi * (f2 + 0.5) * n2 / (2 * T)
    inv = np.concatenate([np.cos(th2), -np.sin(th2)], axis=0) / T
    return jnp.asarray(fwd, bf16), jnp.asarray(inv, bf16)


def _conv_slice(r0, qT_v, kT_v, vT_v, sk_v, coef_v, fwd_ref, inv_ref, aT_v):
    rows = pl.ds(r0, CH)
    k = kT_v[rows, :].astype(f32)
    coef = coef_v[rows, :]
    lane = lax.broadcasted_iota(jnp.int32, (CH, S), 1)
    ks = k * coef[:, 0:1]
    for j in range(1, 4):
        kj = jnp.where(lane >= j, pltpu.roll(k, j, axis=1), 0.0)
        ks = ks + kj * coef[:, j:j + 1]
    u = (ks * vT_v[rows, :].astype(f32)).astype(bf16)
    sk = sk_v[rows, :]
    lhs = jnp.concatenate(
        [u[:, a * T:(a + 1) * T] for a in range(NB)]
        + [sk[:, a * T:(a + 1) * T] for a in range(NB)], axis=0)
    x = jnp.dot(lhs, fwd_ref[...], preferred_element_type=f32)
    flane = lax.broadcasted_iota(jnp.int32, (8, T), 1)
    sgn = jnp.where((flane & 1) == 0, 1.0, -1.0).astype(f32)
    ys = [[None] * (CH // 8) for _ in range(NB)]
    for g in range(CH // 8):
        def blk(a, part, base):
            r = base + a * CH + g * 8
            return x[r:r + 8, part * T:(part + 1) * T]
        ur = [blk(a, 0, 0) for a in range(NB)]
        ui = [blk(a, 1, 0) for a in range(NB)]
        kr = [blk(a, 0, NB * CH) for a in range(NB)]
        ki = [blk(a, 1, NB * CH) for a in range(NB)]
        wr = [sgn * ki[0]] + [kr[a - 1] + sgn * ki[a] for a in range(1, NB)]
        wi = [-(sgn * kr[0])] + [ki[a - 1] - sgn * kr[a] for a in range(1, NB)]
        for a in range(NB):
            yr = wr[0] * ur[a] - wi[0] * ui[a]
            yi = wr[0] * ui[a] + wi[0] * ur[a]
            for dl in range(1, a + 1):
                yr = yr + (wr[dl] * ur[a - dl] - wi[dl] * ui[a - dl])
                yi = yi + (wr[dl] * ui[a - dl] + wi[dl] * ur[a - dl])
            ys[a][g] = jnp.concatenate([yr, yi], axis=1)
    yf = jnp.concatenate([ys[a][g] for a in range(NB) for g in range(CH // 8)], axis=0)
    y = jnp.dot(yf.astype(bf16), inv_ref[...], preferred_element_type=f32)
    y = jnp.concatenate([y[a * CH:(a + 1) * CH, :] for a in range(NB)], axis=1)
    out = qT_v[rows, :].astype(f32) * (y + u.astype(f32) * coef[:, 4:5])
    aT_v[rows, :] = out


def _attention_head(h, q_v, k_s, v_s, ctx_v):
    nq = S // BQ
    row = lax.broadcasted_iota(jnp.int32, (BQ, BQ), 0)
    col = lax.broadcasted_iota(jnp.int32, (BQ, BQ), 1)
    tri = col <= row
    for i in range(nq):
        lo, hi = i * BQ, (i + 1) * BQ
        q = q_v[h, lo:hi, :]
        sd = lax.dot_general(q, k_s[lo:hi, :], NT, preferred_element_type=f32)
        sd = jnp.where(tri, sd, NEG)
        m = jnp.max(sd, axis=1, keepdims=True)
        if i > 0:
            so = lax.dot_general(q, k_s[0:lo, :], NT, preferred_element_type=f32)
            m = jnp.maximum(m, jnp.max(so, axis=1, keepdims=True))
        pd = jnp.exp2(sd - m)
        l = jnp.sum(pd, axis=1, keepdims=True)
        acc = jnp.dot(pd.astype(bf16), v_s[lo:hi, :], preferred_element_type=f32)
        if i > 0:
            po = jnp.exp2(so - m)
            l = l + jnp.sum(po, axis=1, keepdims=True)
            acc = acc + jnp.dot(po.astype(bf16), v_s[0:lo, :], preferred_element_type=f32)
        ctx_v[h, lo:hi, :] = (acc * (1.0 / l)).astype(bf16)


NQSTEP = 8
HPS = H // NQSTEP
CCH = C // NQSTEP


def _kernel(qT_h, kT_h, vT_h, shk_ref, sk_h, d_ref, xT_h, c_h, wq_h, wuk_h, wuv_h, woT_h,
            fwd_ref, inv_ref, out_h,
            qT_v, kT_v, vT_v, sk_v, xT_v, x_v, c_v, wq_raw, wq_p, wuk_raw, wuv_raw, wkv_p,
            q_v, ctx_v, wo_v, aT_v, coef_v, k_s, v_s, o_s,
            sem, sem_w, sem_o):
    cp = pltpu.make_async_copy
    c_x = cp(xT_h, xT_v, sem.at[0])
    c_wq = cp(wq_h, wq_raw, sem.at[1])
    c_c = cp(c_h, c_v, sem.at[2])
    c_k = cp(kT_h, kT_v, sem.at[3])
    c_vv = cp(vT_h, vT_v, sem.at[4])
    c_sk = cp(sk_h, sk_v, sem.at[5])
    c_q = cp(qT_h, qT_v, sem.at[6])
    c_wo = cp(woT_h, wo_v, sem.at[7])

    def w_copies(j):
        rs = pl.ds(pl.multiple_of(j * CCH, CCH), CCH) if not isinstance(j, int) else pl.ds(j * CCH, CCH)
        return (cp(wuk_h.at[rs], wuk_raw.at[rs], sem_w.at[0, j]),
                cp(wuv_h.at[rs], wuv_raw.at[rs], sem_w.at[1, j]))

    c_x.start()
    c_wq.start()
    for j in range(NQSTEP):
        for c in w_copies(j):
            c.start()
    c_c.start()
    c_k.start()
    c_vv.start()
    c_sk.start()
    c_q.start()
    c_wo.start()

    tab = jnp.concatenate([shk_ref[...].astype(f32), d_ref[...].astype(f32).reshape(1, M),
                           jnp.zeros((3, M), f32)], axis=0)
    coef_v[...] = tab.T

    c_x.wait()
    for j in range(S // 512):
        x_v[j * 512:(j + 1) * 512, :] = xT_v[:, j * 512:(j + 1) * 512].T
    c_wq.wait()
    for j in range(M // 64):
        wq_p[:, j * 64:(j + 1) * 64, :] = pltpu.einshape("chd->hcd", wq_raw[j * 64:(j + 1) * 64])

    def qstep(j, carry):
        for c in w_copies(j):
            c.wait()
        for hh in range(HPS):
            h = j * HPS + hh
            qh = jnp.dot(x_v[...], wq_p[h], preferred_element_type=f32)
            q_v[h] = (qh * QSCALE).astype(bf16)
        for t in range(CCH // 64):
            rs = pl.ds(pl.multiple_of(j * CCH + t * 64, 64), 64)
            wkv_p[:, rs, 0:D] = pltpu.einshape("chd->hcd", wuk_raw[rs])
            wkv_p[:, rs, D:2 * D] = pltpu.einshape("chd->hcd", wuv_raw[rs])
        return carry
    lax.fori_loop(0, NQSTEP, qstep, 0)

    c_c.wait()
    c_k.wait()
    c_vv.wait()
    c_sk.wait()
    c_q.wait()
    c_wo.wait()

    def head(h, carry):
        for j in range(S // 512):
            kv = jnp.dot(c_v[j * 512:(j + 1) * 512, :], wkv_p[h], preferred_element_type=f32)
            k_s[j * 512:(j + 1) * 512, :] = kv[:, 0:D].astype(bf16)
            v_s[j * 512:(j + 1) * 512, :] = kv[:, D:2 * D].astype(bf16)
        r0 = pl.multiple_of(jnp.minimum(h * CH, M - CH), CH)
        _conv_slice(r0, qT_v, kT_v, vT_v, sk_v, coef_v, fwd_ref, inv_ref, aT_v)
        _attention_head(h, q_v, k_s, v_s, ctx_v)
        return carry
    lax.fori_loop(0, H, head, 0)

    outs = []
    for j in range(S // BQ):
        lo, hi = j * BQ, (j + 1) * BQ
        bT = lax.dot_general(wo_v[0], ctx_v[0, lo:hi, :], NT, preferred_element_type=f32)
        for h in range(1, H):
            bT = bT + lax.dot_general(wo_v[h], ctx_v[h, lo:hi, :], NT, preferred_element_type=f32)
        full = jnp.concatenate([aT_v[:, lo:hi], bT], axis=0)
        o_s[lo:hi, :] = full.T.astype(bf16)
        oc = cp(o_s.at[lo:hi], out_h.at[lo:hi], sem_o.at[j])
        oc.start()
        outs.append(oc)
    for oc in outs:
        oc.wait()


@jax.jit
def pallas_concat_heads__ssm_conv_h3__compressed_kv_cla__prompt_kernel(
    A_q: jax.Array,
    A_k: jax.Array,
    A_v: jax.Array,
    A_shift_k: jax.Array,
    A_ssm_k: jax.Array,
    A_ssm_D: jax.Array,
    B_x: jax.Array,
    B_c_kv: jax.Array,
    B_w_q: jax.Array,
    B_w_uk: jax.Array,
    B_w_uv: jax.Array,
    B_w_o: jax.Array,
):
    fwd, inv = _dft_mats()
    hbm = pl.BlockSpec(memory_space=pltpu.HBM)
    vmem = pl.BlockSpec(memory_space=pltpu.VMEM)
    V = pltpu.VMEM
    out = pl.pallas_call(
        _kernel,
        out_shape=jax.ShapeDtypeStruct((S, 2 * M), bf16),
        in_specs=[hbm, hbm, hbm, vmem, hbm, vmem, hbm, hbm, hbm, hbm, hbm, hbm, vmem, vmem],
        out_specs=hbm,
        scratch_shapes=[
            V((M, S), bf16), V((M, S), bf16), V((M, S), bf16), V((M, S), bf16),
            V((M, S), bf16), V((S, M), bf16), V((S, C), bf16),
            V((M, H, D), bf16), V((H, M, D), bf16),
            V((C, H, D), bf16), V((C, H, D), bf16), V((H, C, 2 * D), bf16),
            V((H, S, D), bf16), V((H, S, D), bf16),
            V((H, M, D), bf16), V((M, S), f32), V((M, 8), f32),
            V((S, D), bf16), V((S, D), bf16), V((S, 2 * M), bf16),
            pltpu.SemaphoreType.DMA((8,)),
            pltpu.SemaphoreType.DMA((2, NQSTEP)),
            pltpu.SemaphoreType.DMA((S // BQ,)),
        ],
        compiler_params=pltpu.CompilerParams(vmem_limit_bytes=120 * 1024 * 1024),
    )(A_q[0].T, A_k[0].T, A_v[0].T, A_shift_k.T, A_ssm_k, A_ssm_D, B_x[0].T, B_c_kv[0],
      B_w_q, B_w_uk, B_w_uv, jnp.swapaxes(B_w_o, 1, 2), fwd, inv)
    return out[None]
```

```python
import numpy as np
import jax
import jax.numpy as jnp
from jax import lax
import jax.experimental.pallas as pl
import jax.experimental.pallas.tpu as pltpu

f32 = jnp.float32
bf16 = jnp.bfloat16
NT = (((1,), (1,)), ((), ()))

S = 2048
M = 448
H = 16
D = 256
C = 1024
T = 128
NB = S // T
BQ = 256
CH = 32
NEG = -1e30
QSCALE = float(D ** -0.5 * np.log2(np.e))


def _dft_mats():
    n = np.arange(T)[:, None]
    f = np.arange(T)[None, :]
    th = 2 * np.pi * (f + 0.5) * n / (2 * T)
    fwd = np.concatenate([np.cos(th), -np.sin(th)], axis=1)
    n2 = (T + np.arange(T))[None, :]
    f2 = np.arange(T)[:, None]
    th2 = 2 * np.pi * (f2 + 0.5) * n2 / (2 * T)
    inv = np.concatenate([np.cos(th2), -np.sin(th2)], axis=0) / T
    return jnp.asarray(fwd, bf16), jnp.asarray(inv, bf16)


class _Conv:
    def __init__(self, r0, qT_v, kT_v, vT_v, sk_v, coef_v, fwd_ref, inv_ref, aT_v):
        self.rows = pl.ds(r0, CH)
        self.refs = (qT_v, kT_v, vT_v, sk_v, coef_v, fwd_ref, inv_ref, aT_v)
        self.ys = [[None] * (CH // 8) for _ in range(NB)]
        self.w = {}

    def prep(self):
        qT_v, kT_v, vT_v, sk_v, coef_v, fwd_ref, inv_ref, aT_v = self.refs
        rows = self.rows
        k = kT_v[rows, :].astype(f32)
        coef = coef_v[rows, :]
        lane = lax.broadcasted_iota(jnp.int32, (CH, S), 1)
        ks = k * coef[:, 0:1]
        for j in range(1, 4):
            kj = jnp.where(lane >= j, pltpu.roll(k, j, axis=1), 0.0)
            ks = ks + kj * coef[:, j:j + 1]
        self.u = (ks * vT_v[rows, :].astype(f32)).astype(bf16)
        self.dcol = coef[:, 4:5]

    def fwd(self):
        qT_v, kT_v, vT_v, sk_v, coef_v, fwd_ref, inv_ref, aT_v = self.refs
        u = self.u
        sk = sk_v[self.rows, :]
        lhs = jnp.concatenate(
            [u[:, a * T:(a + 1) * T] for a in range(NB)]
            + [sk[:, a * T:(a + 1) * T] for a in range(NB)], axis=0)
        self.x = jnp.dot(lhs, fwd_ref[...], preferred_element_type=f32)

    def _blk(self, g, a, part, base):
        r = base + a * CH + g * 8
        return self.x[r:r + 8, part * T:(part + 1) * T]

    def mac(self, g, alist):
        if g not in self.w:
            flane = lax.broadcasted_iota(jnp.int32, (8, T), 1)
            sgn = jnp.where((flane & 1) == 0, 1.0, -1.0).astype(f32)
            kr = [self._blk(g, a, 0, NB * CH) for a in range(NB)]
            ki = [self._blk(g, a, 1, NB * CH) for a in range(NB)]
            wr = [sgn * ki[0]] + [kr[a - 1] + sgn * ki[a] for a in range(1, NB)]
            wi = [-(sgn * kr[0])] + [ki[a - 1] - sgn * kr[a] for a in range(1, NB)]
            self.w[g] = (wr, wi)
        wr, wi = self.w[g]
        ur = [self._blk(g, a, 0, 0) for a in range(NB)]
        ui = [self._blk(g, a, 1, 0) for a in range(NB)]
        for a in alist:
            yr = wr[0] * ur[a] - wi[0] * ui[a]
            yi = wr[0] * ui[a] + wi[0] * ur[a]
            for dl in range(1, a + 1):
                yr = yr + (wr[dl] * ur[a - dl] - wi[dl] * ui[a - dl])
                yi = yi + (wr[dl] * ui[a - dl] + wi[dl] * ur[a - dl])
            self.ys[a][g] = jnp.concatenate([yr, yi], axis=1)

    def inv(self):
        inv_ref = self.refs[6]
        yf = jnp.concatenate([self.ys[a][g] for a in range(NB) for g in range(CH // 8)], axis=0)
        self.y = jnp.dot(yf.astype(bf16), inv_ref[...], preferred_element_type=f32)

    def gate(self):
        qT_v, aT_v = self.refs[0], self.refs[7]
        y = jnp.concatenate([self.y[a * CH:(a + 1) * CH, :] for a in range(NB)], axis=1)
        aT_v[self.rows, :] = qT_v[self.rows, :].astype(f32) * (y + self.u.astype(f32) * self.dcol)


HB = BQ // 2


def _tiles(x):
    return [x[:, t * 128:(t + 1) * 128] for t in range(x.shape[1] // 128)]


def _fold(op, xs):
    r = xs[0]
    for x in xs[1:]:
        r = op(r, x)
    return r


class _QBlock:
    def __init__(self, h, i, q_v, k_s, v_s, ctx_v):
        self.h, self.i = h, i
        self.q_v, self.k_s, self.v_s, self.ctx_v = q_v, k_s, v_s, ctx_v
        self.lo = i * BQ
        end = self.lo + HB
        self.chunks = [(a, min(a + KCH, end)) for a in range(0, end, KCH)]
        self.s = [None] * len(self.chunks)
        self.p = [None] * len(self.chunks)
        self.mrun = None
        self.lrun = None
        self.acc = None

    def qk(self, c):
        lo = self.lo
        a, b = self.chunks[c]
        q = self.q_v[self.h, lo:lo + BQ, :]
        s = lax.dot_general(q, self.k_s[a:b, :], NT, preferred_element_type=f32)
        ts = _tiles(s)
        if c == len(self.chunks) - 1:
            row = lax.broadcasted_iota(jnp.int32, (BQ, 128), 0)
            col = lax.broadcasted_iota(jnp.int32, (BQ, 128), 1)
            ts[-1] = jnp.where(col <= row, ts[-1], NEG)
            sc = lax.dot_general(q[HB:, :], self.k_s[b:b + HB, :], NT, preferred_element_type=f32)
            row = lax.broadcasted_iota(jnp.int32, (HB, 128), 0)
            col = lax.broadcasted_iota(jnp.int32, (HB, 128), 1)
            self.sc = jnp.where(col <= row, sc, NEG)
        self.s[c] = ts
        m = _fold(jnp.maximum, ts)
        self.mrun = m if self.mrun is None else jnp.maximum(self.mrun, m)

    def rowmax(self):
        mr = jnp.concatenate([self.mrun[:HB], jnp.maximum(self.mrun[HB:], self.sc)], axis=0)
        self.m = jnp.max(mr, axis=1, keepdims=True)

    def exp(self, c):
        ps = [jnp.exp2(t - self.m) for t in self.s[c]]
        l = _fold(jnp.add, ps)
        if c == len(self.chunks) - 1:
            pc = jnp.exp2(self.sc - self.m[HB:])
            l = jnp.concatenate([l[:HB], l[HB:] + pc], axis=0)
            self.pc = pc.astype(bf16)
        self.lrun = l if self.lrun is None else self.lrun + l
        self.p[c] = jnp.concatenate([p.astype(bf16) for p in ps], axis=1)

    def pv(self, c):
        a, b = self.chunks[c]
        r = jnp.dot(self.p[c], self.v_s[a:b, :], preferred_element_type=f32)
        self.acc = r if self.acc is None else self.acc + r
        if c == len(self.chunks) - 1:
            rc = jnp.dot(self.pc, self.v_s[b:b + HB, :], preferred_element_type=f32)
            self.acc = jnp.concatenate([self.acc[:HB], self.acc[HB:] + rc], axis=0)

    def finish(self):
        l = jnp.sum(self.lrun, axis=1, keepdims=True)
        self.ctx_v[self.h, self.lo:self.lo + BQ, :] = (self.acc * (1.0 / l)).astype(bf16)


KCH = 512


def _head_body(h, c_v, wkv_p, k_s, v_s, q_v, ctx_v, conv):
    nq = S // BQ

    def proj(j, half):
        dst = k_s if half == 0 else v_s
        r = jnp.dot(c_v[j * BQ:(j + 1) * BQ, :], wkv_p[h, :, half * D:(half + 1) * D],
                    preferred_element_type=f32)
        dst[j * BQ:(j + 1) * BQ, :] = r.astype(bf16)

    blocks = [_QBlock(h, i, q_v, k_s, v_s, ctx_v) for i in range(nq)]
    parts = [list(range(0, 9)), list(range(9, 13)), list(range(13, 16))]
    macs = [(g, p) for g in range(CH // 8) for p in parts]

    def take_mac():
        if macs:
            conv.mac(*macs.pop(0))

    proj(0, 0)
    conv.prep()
    proj(0, 1)
    conv.fwd()
    proj(1, 0)
    for c in range(len(blocks[0].chunks)):
        blocks[0].qk(c)
    proj(1, 1)
    blocks[0].rowmax()
    for i in range(nq):
        cur = blocks[i]
        nxt = blocks[i + 1] if i + 1 < nq else None
        n = len(cur.chunks)
        nn = len(nxt.chunks) if nxt else 0
        for c in range(max(n, nn)):
            if c < nn:
                nxt.qk(c)
            if c < n:
                cur.exp(c)
        if i + 2 < nq:
            proj(i + 2, 0)
            take_mac()
        if nxt:
            nxt.rowmax()
        for c in range(n):
            cur.pv(c)
        if i + 2 < nq:
            take_mac()
            proj(i + 2, 1)
        cur.finish()
        if i == nq - 3:
            assert not macs
            conv.inv()
            conv.gate()


NQSTEP = 8
HPS = H // NQSTEP
CCH = C // NQSTEP


def _kernel(qT_h, kT_h, vT_h, shk_ref, sk_h, d_ref, xT_h, c_h, wq_h, wuk_h, wuv_h, woT_h,
            fwd_ref, inv_ref, out_h,
            qT_v, kT_v, vT_v, sk_v, xT_v, x_v, c_v, wq_raw, wq_p, wuk_raw, wuv_raw, wkv_p,
            q_v, ctx_v, wo_v, aT_v, coef_v, k_s, v_s, o_s,
            sem, sem_w, sem_o):
    cp = pltpu.make_async_copy
    c_x = cp(xT_h, xT_v, sem.at[0])
    c_wq = cp(wq_h, wq_raw, sem.at[1])
    c_c = cp(c_h, c_v, sem.at[2])
    c_k = cp(kT_h, kT_v, sem.at[3])
    c_vv = cp(vT_h, vT_v, sem.at[4])
    c_sk = cp(sk_h, sk_v, sem.at[5])
    c_q = cp(qT_h, qT_v, sem.at[6])
    c_wo = cp(woT_h, wo_v, sem.at[7])

    def w_copies(j):
        rs = pl.ds(pl.multiple_of(j * CCH, CCH), CCH) if not isinstance(j, int) else pl.ds(j * CCH, CCH)
        return (cp(wuk_h.at[rs], wuk_raw.at[rs], sem_w.at[0, j]),
                cp(wuv_h.at[rs], wuv_raw.at[rs], sem_w.at[1, j]))

    c_x.start()
    c_wq.start()

    tab = jnp.concatenate([shk_ref[...].astype(f32), d_ref[...].astype(f32).reshape(1, M),
                           jnp.zeros((3, M), f32)], axis=0)
    coef_v[...] = tab.T

    c_x.wait()
    for j in range(S // 512):
        x_v[j * 512:(j + 1) * 512, :] = xT_v[:, j * 512:(j + 1) * 512].T
    c_wq.wait()
    for j in range(NQSTEP):
        for c in w_copies(j):
            c.start()
    c_c.start()
    c_k.start()
    c_vv.start()
    c_sk.start()
    c_q.start()
    c_wo.start()
    for j in range(M // 64):
        wq_p[:, j * 64:(j + 1) * 64, :] = pltpu.einshape("chd->hcd", wq_raw[j * 64:(j + 1) * 64])

    def qstep(j, carry):
        for c in w_copies(j):
            c.wait()
        for hh in range(HPS):
            h = j * HPS + hh
            qh = jnp.dot(x_v[...], wq_p[h], preferred_element_type=f32)
            q_v[h] = (qh * QSCALE).astype(bf16)
        for t in range(CCH // 64):
            rs = pl.ds(pl.multiple_of(j * CCH + t * 64, 64), 64)
            wkv_p[:, rs, 0:D] = pltpu.einshape("chd->hcd", wuk_raw[rs])
            wkv_p[:, rs, D:2 * D] = pltpu.einshape("chd->hcd", wuv_raw[rs])
        return carry
    lax.fori_loop(0, NQSTEP, qstep, 0)

    c_c.wait()
    c_k.wait()
    c_vv.wait()
    c_sk.wait()
    c_q.wait()
    c_wo.wait()

    def head(h, carry):
        r0 = pl.multiple_of(jnp.minimum(h * CH, M - CH), CH)
        conv = _Conv(r0, qT_v, kT_v, vT_v, sk_v, coef_v, fwd_ref, inv_ref, aT_v)
        _head_body(h, c_v, wkv_p, k_s, v_s, q_v, ctx_v, conv)
        return carry
    lax.fori_loop(0, H, head, 0)

    def ostep(j, carry):
        rs = pl.ds(pl.multiple_of(j * BQ, BQ), BQ)
        bT = lax.dot_general(wo_v[0], ctx_v[0, rs, :], NT, preferred_element_type=f32)
        for h in range(1, H):
            bT = bT + lax.dot_general(wo_v[h], ctx_v[h, rs, :], NT, preferred_element_type=f32)
        full = jnp.concatenate([aT_v[:, rs], bT], axis=0)
        o_s[rs, :] = full.T.astype(bf16)
        cp(o_s.at[rs], out_h.at[rs], sem_o.at[j]).start()
        return carry
    lax.fori_loop(0, S // BQ, ostep, 0)
    for j in range(S // BQ):
        cp(o_s.at[j * BQ:(j + 1) * BQ], out_h.at[j * BQ:(j + 1) * BQ], sem_o.at[j]).wait()


@jax.jit
def pallas_concat_heads__ssm_conv_h3__compressed_kv_cla__prompt_kernel(
    A_q: jax.Array,
    A_k: jax.Array,
    A_v: jax.Array,
    A_shift_k: jax.Array,
    A_ssm_k: jax.Array,
    A_ssm_D: jax.Array,
    B_x: jax.Array,
    B_c_kv: jax.Array,
    B_w_q: jax.Array,
    B_w_uk: jax.Array,
    B_w_uv: jax.Array,
    B_w_o: jax.Array,
):
    fwd, inv = _dft_mats()
    hbm = pl.BlockSpec(memory_space=pltpu.HBM)
    vmem = pl.BlockSpec(memory_space=pltpu.VMEM)
    V = pltpu.VMEM
    out = pl.pallas_call(
        _kernel,
        out_shape=jax.ShapeDtypeStruct((S, 2 * M), bf16),
        in_specs=[hbm, hbm, hbm, vmem, hbm, vmem, hbm, hbm, hbm, hbm, hbm, hbm, vmem, vmem],
        out_specs=hbm,
        scratch_shapes=[
            V((M, S), bf16), V((M, S), bf16), V((M, S), bf16), V((M, S), bf16),
            V((M, S), bf16), V((S, M), bf16), V((S, C), bf16),
            V((M, H, D), bf16), V((H, M, D), bf16),
            V((C, H, D), bf16), V((C, H, D), bf16), V((H, C, 2 * D), bf16),
            V((H, S, D), bf16), V((H, S, D), bf16),
            V((H, M, D), bf16), V((M, S), f32), V((M, 8), f32),
            V((S, D), bf16), V((S, D), bf16), V((S, 2 * M), bf16),
            pltpu.SemaphoreType.DMA((8,)),
            pltpu.SemaphoreType.DMA((2, NQSTEP)),
            pltpu.SemaphoreType.DMA((S // BQ,)),
        ],
        compiler_params=pltpu.CompilerParams(vmem_limit_bytes=120 * 1024 * 1024),
    )(A_q[0].T, A_k[0].T, A_v[0].T, A_shift_k.T, A_ssm_k, A_ssm_D, B_x[0].T, B_c_kv[0],
      B_w_q, B_w_uk, B_w_uv, jnp.swapaxes(B_w_o, 1, 2), fwd, inv)
    return out[None]
```

```python
import numpy as np
import jax
import jax.numpy as jnp
from jax import lax
import jax.experimental.pallas as pl
import jax.experimental.pallas.tpu as pltpu

f32 = jnp.float32
bf16 = jnp.bfloat16
NT = (((1,), (1,)), ((), ()))

S = 2048
M = 448
H = 16
D = 256
C = 1024
T = 128
NB = S // T
BQ = 256
CH = 32
NEG = -1e30
QSCALE = float(D ** -0.5 * np.log2(np.e))


def _dft_mats():
    n = np.arange(T)[:, None]
    f = np.arange(T)[None, :]
    th = 2 * np.pi * (f + 0.5) * n / (2 * T)
    fwd = np.concatenate([np.cos(th), -np.sin(th)], axis=1)
    n2 = (T + np.arange(T))[None, :]
    f2 = np.arange(T)[:, None]
    th2 = 2 * np.pi * (f2 + 0.5) * n2 / (2 * T)
    inv = np.concatenate([np.cos(th2), -np.sin(th2)], axis=0) / T
    return jnp.asarray(fwd, bf16), jnp.asarray(inv, bf16)


class _Conv:
    def __init__(self, r0, qT_v, kT_v, vT_v, sk_v, coef_v, fwd_ref, inv_ref, aT_v):
        self.rows = pl.ds(r0, CH)
        self.refs = (qT_v, kT_v, vT_v, sk_v, coef_v, fwd_ref, inv_ref, aT_v)
        self.ys = [[None] * (CH // 8) for _ in range(NB)]
        self.w = {}
        self.yt = [None] * (CH // 8)

    def prep(self):
        qT_v, kT_v, vT_v, sk_v, coef_v, fwd_ref, inv_ref, aT_v = self.refs
        rows = self.rows
        k = kT_v[rows, :].astype(f32)
        coef = coef_v[rows, :]
        lane = lax.broadcasted_iota(jnp.int32, (CH, S), 1)
        ks = k * coef[:, 0:1]
        for j in range(1, 4):
            kj = jnp.where(lane >= j, pltpu.roll(k, j, axis=1), 0.0)
            ks = ks + kj * coef[:, j:j + 1]
        self.u = (ks * vT_v[rows, :].astype(f32)).astype(bf16)
        self.dcol = coef[:, 4:5]

    def fwd(self):
        qT_v, kT_v, vT_v, sk_v, coef_v, fwd_ref, inv_ref, aT_v = self.refs
        u = self.u
        sk = sk_v[self.rows, :]
        lhs = jnp.concatenate(
            [u[:, a * T:(a + 1) * T] for a in range(NB)]
            + [sk[:, a * T:(a + 1) * T] for a in range(NB)], axis=0)
        self.x = jnp.dot(lhs, fwd_ref[...], preferred_element_type=f32)

    def _blk(self, g, a, part, base):
        r = base + a * CH + g * 8
        return self.x[r:r + 8, part * T:(part + 1) * T]

    def mac(self, g, alist):
        if g not in self.w:
            flane = lax.broadcasted_iota(jnp.int32, (8, T), 1)
            sgn = jnp.where((flane & 1) == 0, 1.0, -1.0).astype(f32)
            kr = [self._blk(g, a, 0, NB * CH) for a in range(NB)]
            ki = [self._blk(g, a, 1, NB * CH) for a in range(NB)]
            wr = [sgn * ki[0]] + [kr[a - 1] + sgn * ki[a] for a in range(1, NB)]
            wi = [-(sgn * kr[0])] + [ki[a - 1] - sgn * kr[a] for a in range(1, NB)]
            self.w[g] = (wr, wi)
        wr, wi = self.w[g]
        ur = [self._blk(g, a, 0, 0) for a in range(NB)]
        ui = [self._blk(g, a, 1, 0) for a in range(NB)]
        for a in alist:
            yr = wr[0] * ur[a] - wi[0] * ui[a]
            yi = wr[0] * ui[a] + wi[0] * ur[a]
            for dl in range(1, a + 1):
                yr = yr + (wr[dl] * ur[a - dl] - wi[dl] * ui[a - dl])
                yi = yi + (wr[dl] * ui[a - dl] + wi[dl] * ur[a - dl])
            self.ys[a][g] = jnp.concatenate([yr, yi], axis=1)

    def inv(self, g):
        qT_v, inv_ref, aT_v = self.refs[0], self.refs[6], self.refs[7]
        yf = jnp.concatenate([self.ys[a][g] for a in range(NB)], axis=0)
        y = jnp.dot(yf.astype(bf16), inv_ref[...], preferred_element_type=f32)
        self.yt[g] = jnp.concatenate([y[a * 8:(a + 1) * 8, :] for a in range(NB)], axis=1)

    def gate(self):
        qT_v, aT_v = self.refs[0], self.refs[7]
        y = jnp.concatenate(self.yt, axis=0)
        aT_v[self.rows, :] = qT_v[self.rows, :].astype(f32) * (y + self.u.astype(f32) * self.dcol)


HB = BQ // 2


def _tiles(x):
    return [x[:, t * 128:(t + 1) * 128] for t in range(x.shape[1] // 128)]


def _fold(op, xs):
    r = xs[0]
    for x in xs[1:]:
        r = op(r, x)
    return r


class _QBlock:
    def __init__(self, h, i, q_v, k_s, v_s, ctx_v):
        self.h, self.i = h, i
        self.q_v, self.k_s, self.v_s, self.ctx_v = q_v, k_s, v_s, ctx_v
        self.lo = i * BQ
        end = self.lo + HB
        self.chunks = [(a, min(a + KCH, end)) for a in range(0, end, KCH)]
        self.s = [None] * len(self.chunks)
        self.p = [None] * len(self.chunks)
        self.mrun = None
        self.lrun = None
        self.acc = None

    def qk(self, c):
        lo = self.lo
        a, b = self.chunks[c]
        q = self.q_v[self.h, lo:lo + BQ, :]
        s = lax.dot_general(q, self.k_s[a:b, :], NT, preferred_element_type=f32)
        ts = _tiles(s)
        if c == len(self.chunks) - 1:
            row = lax.broadcasted_iota(jnp.int32, (BQ, 128), 0)
            col = lax.broadcasted_iota(jnp.int32, (BQ, 128), 1)
            ts[-1] = jnp.where(col <= row, ts[-1], NEG)
            sc = lax.dot_general(q[HB:, :], self.k_s[b:b + HB, :], NT, preferred_element_type=f32)
            row = lax.broadcasted_iota(jnp.int32, (HB, 128), 0)
            col = lax.broadcasted_iota(jnp.int32, (HB, 128), 1)
            self.sc = jnp.where(col <= row, sc, NEG)
        self.s[c] = ts
        m = _fold(jnp.maximum, ts)
        self.mrun = m if self.mrun is None else jnp.maximum(self.mrun, m)

    def stats(self):
        mr = jnp.concatenate([self.mrun[:HB], jnp.maximum(self.mrun[HB:], self.sc)], axis=0)
        m = jnp.max(mr, axis=1, keepdims=True)
        l = _fold(jnp.add, [jnp.exp2(t - m) for ts in self.s for t in ts])
        l = jnp.concatenate([l[:HB], l[HB:] + jnp.exp2(self.sc - m[HB:])], axis=0)
        self.off = m + jnp.log2(jnp.sum(l, axis=1, keepdims=True))

    def pv(self, c):
        a, b = self.chunks[c]
        p = jnp.concatenate([jnp.exp2(t - self.off) for t in self.s[c]], axis=1).astype(bf16)
        r = jnp.dot(p, self.v_s[a:b, :], preferred_element_type=f32)
        self.acc = r if self.acc is None else self.acc + r
        if c == len(self.chunks) - 1:
            pc = jnp.exp2(self.sc - self.off[HB:]).astype(bf16)
            rc = jnp.dot(pc, self.v_s[b:b + HB, :], preferred_element_type=f32)
            self.acc = jnp.concatenate([self.acc[:HB], self.acc[HB:] + rc], axis=0)

    def finish(self):
        self.ctx_v[self.h, self.lo:self.lo + BQ, :] = self.acc.astype(bf16)


KCH = 512


def _head_body(h, c_v, wkv_p, k_s, v_s, q_v, ctx_v, conv):
    nq = S // BQ

    def proj(j, half):
        dst = k_s if half == 0 else v_s
        r = jnp.dot(c_v[j * BQ:(j + 1) * BQ, :], wkv_p[h, :, half * D:(half + 1) * D],
                    preferred_element_type=f32)
        dst[j * BQ:(j + 1) * BQ, :] = r.astype(bf16)

    blocks = [_QBlock(h, i, q_v, k_s, v_s, ctx_v) for i in range(nq)]
    proj(0, 0)
    conv.prep()
    proj(0, 1)
    conv.fwd()
    proj(1, 0)
    for c in range(len(blocks[0].chunks)):
        blocks[0].qk(c)
    proj(1, 1)
    for i in range(nq):
        cur = blocks[i]
        nxt = blocks[i + 1] if i + 1 < nq else None
        if nxt:
            for c in range(len(nxt.chunks)):
                nxt.qk(c)
        if i + 2 < nq:
            proj(i + 2, 0)
        cur.stats()
        for c in range(len(cur.chunks)):
            cur.pv(c)
        cur.finish()
        if i + 2 < nq:
            proj(i + 2, 1)
        if i < CH // 8:
            conv.mac(i, list(range(NB)))
            conv.inv(i)
        if i == CH // 8:
            conv.gate()


NQSTEP = 8
HPS = H // NQSTEP
CCH = C // NQSTEP


def _kernel(qT_h, kT_h, vT_h, shk_ref, sk_h, d_ref, xT_h, c_h, wq_h, wuk_h, wuv_h, woT_h,
            fwd_ref, inv_ref, out_h,
            qT_v, kT_v, vT_v, sk_v, xT_v, x_v, c_v, wq_raw, wq_p, wuk_raw, wuv_raw, wkv_p,
            q_v, ctx_v, wo_v, aT_v, coef_v, k_s, v_s, o_s,
            sem, sem_w, sem_o):
    cp = pltpu.make_async_copy
    c_x = cp(xT_h, xT_v, sem.at[0])
    c_wq = cp(wq_h, wq_raw, sem.at[1])
    c_c = cp(c_h, c_v, sem.at[2])
    c_k = cp(kT_h, kT_v, sem.at[3])
    c_vv = cp(vT_h, vT_v, sem.at[4])
    c_sk = cp(sk_h, sk_v, sem.at[5])
    c_q = cp(qT_h, qT_v, sem.at[6])
    c_wo = cp(woT_h, wo_v, sem.at[7])

    def w_copies(j):
        rs = pl.ds(pl.multiple_of(j * CCH, CCH), CCH) if not isinstance(j, int) else pl.ds(j * CCH, CCH)
        return (cp(wuk_h.at[rs], wuk_raw.at[rs], sem_w.at[0, j]),
                cp(wuv_h.at[rs], wuv_raw.at[rs], sem_w.at[1, j]))

    c_x.start()
    c_wq.start()

    tab = jnp.concatenate([shk_ref[...].astype(f32), d_ref[...].astype(f32).reshape(1, M),
                           jnp.zeros((3, M), f32)], axis=0)
    coef_v[...] = tab.T

    c_x.wait()
    for j in range(S // 512):
        x_v[j * 512:(j + 1) * 512, :] = xT_v[:, j * 512:(j + 1) * 512].T
    c_wq.wait()
    for j in range(NQSTEP):
        for c in w_copies(j):
            c.start()
    c_c.start()
    c_k.start()
    c_vv.start()
    c_sk.start()
    c_q.start()
    c_wo.start()
    for j in range(M // 64):
        wq_p[:, j * 64:(j + 1) * 64, :] = pltpu.einshape("chd->hcd", wq_raw[j * 64:(j + 1) * 64])

    def qstep(j, carry):
        for c in w_copies(j):
            c.wait()
        for hh in range(HPS):
            h = j * HPS + hh
            qh = jnp.dot(x_v[...], wq_p[h], preferred_element_type=f32)
            q_v[h] = (qh * QSCALE).astype(bf16)
        for t in range(CCH // 64):
            rs = pl.ds(pl.multiple_of(j * CCH + t * 64, 64), 64)
            wkv_p[:, rs, 0:D] = pltpu.einshape("chd->hcd", wuk_raw[rs])
            wkv_p[:, rs, D:2 * D] = pltpu.einshape("chd->hcd", wuv_raw[rs])
        return carry
    lax.fori_loop(0, NQSTEP, qstep, 0)

    c_c.wait()
    c_k.wait()
    c_vv.wait()
    c_sk.wait()
    c_q.wait()
    c_wo.wait()

    def head(h, carry):
        r0 = pl.multiple_of(jnp.minimum(h * CH, M - CH), CH)
        conv = _Conv(r0, qT_v, kT_v, vT_v, sk_v, coef_v, fwd_ref, inv_ref, aT_v)
        _head_body(h, c_v, wkv_p, k_s, v_s, q_v, ctx_v, conv)
        return carry
    lax.fori_loop(0, H, head, 0)

    def ostep(j, carry):
        rs = pl.ds(pl.multiple_of(j * BQ, BQ), BQ)
        bT = lax.dot_general(wo_v[0], ctx_v[0, rs, :], NT, preferred_element_type=f32)
        for h in range(1, H):
            bT = bT + lax.dot_general(wo_v[h], ctx_v[h, rs, :], NT, preferred_element_type=f32)
        full = jnp.concatenate([aT_v[:, rs], bT], axis=0)
        o_s[rs, :] = full.T.astype(bf16)
        cp(o_s.at[rs], out_h.at[rs], sem_o.at[j]).start()
        return carry
    lax.fori_loop(0, S // BQ, ostep, 0)
    for j in range(S // BQ):
        cp(o_s.at[j * BQ:(j + 1) * BQ], out_h.at[j * BQ:(j + 1) * BQ], sem_o.at[j]).wait()


@jax.jit
def pallas_concat_heads__ssm_conv_h3__compressed_kv_cla__prompt_kernel(
    A_q: jax.Array,
    A_k: jax.Array,
    A_v: jax.Array,
    A_shift_k: jax.Array,
    A_ssm_k: jax.Array,
    A_ssm_D: jax.Array,
    B_x: jax.Array,
    B_c_kv: jax.Array,
    B_w_q: jax.Array,
    B_w_uk: jax.Array,
    B_w_uv: jax.Array,
    B_w_o: jax.Array,
):
    fwd, inv = _dft_mats()
    hbm = pl.BlockSpec(memory_space=pltpu.HBM)
    vmem = pl.BlockSpec(memory_space=pltpu.VMEM)
    V = pltpu.VMEM
    out = pl.pallas_call(
        _kernel,
        out_shape=jax.ShapeDtypeStruct((S, 2 * M), bf16),
        in_specs=[hbm, hbm, hbm, vmem, hbm, vmem, hbm, hbm, hbm, hbm, hbm, hbm, vmem, vmem],
        out_specs=hbm,
        scratch_shapes=[
            V((M, S), bf16), V((M, S), bf16), V((M, S), bf16), V((M, S), bf16),
            V((M, S), bf16), V((S, M), bf16), V((S, C), bf16),
            V((M, H, D), bf16), V((H, M, D), bf16),
            V((C, H, D), bf16), V((C, H, D), bf16), V((H, C, 2 * D), bf16),
            V((H, S, D), bf16), V((H, S, D), bf16),
            V((H, M, D), bf16), V((M, S), f32), V((M, 8), f32),
            V((S, D), bf16), V((S, D), bf16), V((S, 2 * M), bf16),
            pltpu.SemaphoreType.DMA((8,)),
            pltpu.SemaphoreType.DMA((2, NQSTEP)),
            pltpu.SemaphoreType.DMA((S // BQ,)),
        ],
        compiler_params=pltpu.CompilerParams(vmem_limit_bytes=120 * 1024 * 1024),
    )(A_q[0].T, A_k[0].T, A_v[0].T, A_shift_k.T, A_ssm_k, A_ssm_D, B_x[0].T, B_c_kv[0],
      B_w_q, B_w_uk, B_w_uv, jnp.swapaxes(B_w_o, 1, 2), fwd, inv)
    return out[None]
```

```python
import numpy as np
import jax
import jax.numpy as jnp
from jax import lax
import jax.experimental.pallas as pl
import jax.experimental.pallas.tpu as pltpu

f32 = jnp.float32
bf16 = jnp.bfloat16
NT = (((1,), (1,)), ((), ()))

S = 2048
M = 448
H = 16
D = 256
C = 1024
T = 128
NB = S // T
BQ = 256
CH = 32
NEG = -1e30
QSCALE = float(D ** -0.5 * np.log2(np.e))


def _dft_mats():
    n = np.arange(T)[:, None]
    f = np.arange(T)[None, :]
    th = 2 * np.pi * (f + 0.5) * n / (2 * T)
    fwd = np.concatenate([np.cos(th), -np.sin(th)], axis=1)
    n2 = (T + np.arange(T))[None, :]
    f2 = np.arange(T)[:, None]
    th2 = 2 * np.pi * (f2 + 0.5) * n2 / (2 * T)
    inv = np.concatenate([np.cos(th2), -np.sin(th2)], axis=0) / T
    return jnp.asarray(fwd, bf16), jnp.asarray(inv, bf16)


class _Conv:
    def __init__(self, r0, qT_v, kT_v, vT_v, sk_v, coef_v, fwd_ref, inv_ref, aT_v):
        self.rows = pl.ds(r0, CH)
        self.refs = (qT_v, kT_v, vT_v, sk_v, coef_v, fwd_ref, inv_ref, aT_v)
        self.ys = [[None] * (CH // 8) for _ in range(NB)]
        self.w = {}
        self.yt = [None] * (CH // 8)

    def prep(self):
        qT_v, kT_v, vT_v, sk_v, coef_v, fwd_ref, inv_ref, aT_v = self.refs
        rows = self.rows
        k = kT_v[rows, :].astype(f32)
        coef = coef_v[rows, :]
        lane = lax.broadcasted_iota(jnp.int32, (CH, S), 1)
        ks = k * coef[:, 0:1]
        for j in range(1, 4):
            kj = jnp.where(lane >= j, pltpu.roll(k, j, axis=1), 0.0)
            ks = ks + kj * coef[:, j:j + 1]
        self.u = (ks * vT_v[rows, :].astype(f32)).astype(bf16)
        self.dcol = coef[:, 4:5]

    def fwd(self):
        qT_v, kT_v, vT_v, sk_v, coef_v, fwd_ref, inv_ref, aT_v = self.refs
        u = self.u
        sk = sk_v[self.rows, :]
        lhs = jnp.concatenate(
            [u[:, a * T:(a + 1) * T] for a in range(NB)]
            + [sk[:, a * T:(a + 1) * T] for a in range(NB)], axis=0)
        self.x = jnp.dot(lhs, fwd_ref[...], preferred_element_type=f32)

    def _blk(self, g, a, part, base):
        r = base + a * CH + g * 8
        return self.x[r:r + 8, part * T:(part + 1) * T]

    def mac(self, g, alist):
        if g not in self.w:
            flane = lax.broadcasted_iota(jnp.int32, (8, T), 1)
            sgn = jnp.where((flane & 1) == 0, 1.0, -1.0).astype(f32)
            kr = [self._blk(g, a, 0, NB * CH) for a in range(NB)]
            ki = [self._blk(g, a, 1, NB * CH) for a in range(NB)]
            wr = [sgn * ki[0]] + [kr[a - 1] + sgn * ki[a] for a in range(1, NB)]
            wi = [-(sgn * kr[0])] + [ki[a - 1] - sgn * kr[a] for a in range(1, NB)]
            self.w[g] = (wr, wi)
        wr, wi = self.w[g]
        ur = [self._blk(g, a, 0, 0) for a in range(NB)]
        ui = [self._blk(g, a, 1, 0) for a in range(NB)]
        for a in alist:
            yr = wr[0] * ur[a] - wi[0] * ui[a]
            yi = wr[0] * ui[a] + wi[0] * ur[a]
            for dl in range(1, a + 1):
                yr = yr + (wr[dl] * ur[a - dl] - wi[dl] * ui[a - dl])
                yi = yi + (wr[dl] * ui[a - dl] + wi[dl] * ur[a - dl])
            self.ys[a][g] = jnp.concatenate([yr, yi], axis=1)

    def inv(self, g):
        qT_v, inv_ref, aT_v = self.refs[0], self.refs[6], self.refs[7]
        yf = jnp.concatenate([self.ys[a][g] for a in range(NB)], axis=0)
        y = jnp.dot(yf.astype(bf16), inv_ref[...], preferred_element_type=f32)
        self.yt[g] = jnp.concatenate([y[a * 8:(a + 1) * 8, :] for a in range(NB)], axis=1)

    def gate(self):
        qT_v, aT_v = self.refs[0], self.refs[7]
        y = jnp.concatenate(self.yt, axis=0)
        aT_v[self.rows, :] = qT_v[self.rows, :].astype(f32) * (y + self.u.astype(f32) * self.dcol)


HB = BQ // 2


def _tiles(x):
    return [x[:, t * 128:(t + 1) * 128] for t in range(x.shape[1] // 128)]


def _fold(op, xs):
    r = xs[0]
    for x in xs[1:]:
        r = op(r, x)
    return r


class _QBlock:
    def __init__(self, h, i, q_v, k_s, v_s, ctx_v):
        self.h, self.i = h, i
        self.q_v, self.k_s, self.v_s, self.ctx_v = q_v, k_s, v_s, ctx_v
        self.lo = i * BQ
        end = self.lo + HB
        self.chunks = [(a, min(a + KCH, end)) for a in range(0, end, KCH)]
        self.s = [None] * len(self.chunks)
        self.p = [None] * len(self.chunks)
        self.mrun = None
        self.lrun = None
        self.acc = None

    def qk(self, c):
        lo = self.lo
        a, b = self.chunks[c]
        q = self.q_v[self.h, lo:lo + BQ, :]
        s = lax.dot_general(q, self.k_s[a:b, :], NT, preferred_element_type=f32)
        ts = _tiles(s)
        if c == len(self.chunks) - 1:
            row = lax.broadcasted_iota(jnp.int32, (BQ, 128), 0)
            col = lax.broadcasted_iota(jnp.int32, (BQ, 128), 1)
            ts[-1] = jnp.where(col <= row, ts[-1], NEG)
            sc = lax.dot_general(q[HB:, :], self.k_s[b:b + HB, :], NT, preferred_element_type=f32)
            row = lax.broadcasted_iota(jnp.int32, (HB, 128), 0)
            col = lax.broadcasted_iota(jnp.int32, (HB, 128), 1)
            self.sc = jnp.where(col <= row, sc, NEG)
        self.s[c] = ts
        m = _fold(jnp.maximum, ts)
        self.mrun = m if self.mrun is None else jnp.maximum(self.mrun, m)

    def stats(self):
        mr = jnp.concatenate([self.mrun[:HB], jnp.maximum(self.mrun[HB:], self.sc)], axis=0)
        m = jnp.max(mr, axis=1, keepdims=True)
        l = _fold(jnp.add, [jnp.exp2(t - m) for ts in self.s for t in ts])
        l = jnp.concatenate([l[:HB], l[HB:] + jnp.exp2(self.sc - m[HB:])], axis=0)
        self.off = m + jnp.log2(jnp.sum(l, axis=1, keepdims=True))

    def pv(self, c):
        a, b = self.chunks[c]
        p = jnp.concatenate([jnp.exp2(t - self.off) for t in self.s[c]], axis=1).astype(bf16)
        r = jnp.dot(p, self.v_s[a:b, :], preferred_element_type=f32)
        self.acc = r if self.acc is None else self.acc + r
        if c == len(self.chunks) - 1:
            pc = jnp.exp2(self.sc - self.off[HB:]).astype(bf16)
            rc = jnp.dot(pc, self.v_s[b:b + HB, :], preferred_element_type=f32)
            self.acc = jnp.concatenate([self.acc[:HB], self.acc[HB:] + rc], axis=0)

    def finish(self):
        self.ctx_v[self.h, self.lo:self.lo + BQ, :] = self.acc.astype(bf16)


KCH = 512


def _head_body(h, c_v, wkv_p, k_s, v_s, q_v, ctx_v, conv):
    nq = S // BQ

    def proj(j, half):
        dst = k_s if half == 0 else v_s
        r = jnp.dot(c_v[j * BQ:(j + 1) * BQ, :], wkv_p[H + h, half * C:(half + 1) * C, :],
                    preferred_element_type=f32)
        dst[j * BQ:(j + 1) * BQ, :] = r.astype(bf16)

    blocks = [_QBlock(h, i, q_v, k_s, v_s, ctx_v) for i in range(nq)]
    proj(0, 0)
    conv.prep()
    proj(0, 1)
    conv.fwd()
    proj(1, 0)
    for c in range(len(blocks[0].chunks)):
        blocks[0].qk(c)
    proj(1, 1)
    for i in range(nq):
        cur = blocks[i]
        nxt = blocks[i + 1] if i + 1 < nq else None
        if nxt:
            for c in range(len(nxt.chunks)):
                nxt.qk(c)
        if i + 2 < nq:
            proj(i + 2, 0)
        cur.stats()
        for c in range(len(cur.chunks)):
            cur.pv(c)
        cur.finish()
        if i + 2 < nq:
            proj(i + 2, 1)
        if i < CH // 8:
            conv.mac(i, list(range(NB)))
            conv.inv(i)
        if i == CH // 8:
            conv.gate()


NQSTEP = 8
HPS = H // NQSTEP
RP = 16
CCH = C // NQSTEP


def _kernel(qT_h, kT_h, vT_h, shk_ref, sk_h, d_ref, xT_h, c_h, wq_h, wuk_h, wuv_h, woT_h,
            fwd_ref, inv_ref, out_h,
            qT_v, kT_v, vT_v, sk_v, xT_v, x_v, c_v, wq_raw, wq_p, wuk_raw, wuv_raw,
            qw_v, ctx_v, wo_v, aT_v, coef_v, k_s, v_s, o_s,
            sem, sem_w, sem_o):
    cp = pltpu.make_async_copy
    c_x = cp(xT_h, xT_v, sem.at[0])
    c_wq = cp(wq_h, wq_raw, sem.at[1])
    c_c = cp(c_h, c_v, sem.at[2])
    c_k = cp(kT_h, kT_v, sem.at[3])
    c_vv = cp(vT_h, vT_v, sem.at[4])
    c_sk = cp(sk_h, sk_v, sem.at[5])
    c_q = cp(qT_h, qT_v, sem.at[6])
    c_wo = cp(woT_h, wo_v, sem.at[7])

    def w_copies(j):
        rs = pl.ds(pl.multiple_of(j * CCH, CCH), CCH) if not isinstance(j, int) else pl.ds(j * CCH, CCH)
        return (cp(wuk_h.at[rs], wuk_raw.at[rs], sem_w.at[0, j]),
                cp(wuv_h.at[rs], wuv_raw.at[rs], sem_w.at[1, j]))

    c_x.start()
    c_wq.start()

    tab = jnp.concatenate([shk_ref[...].astype(f32), d_ref[...].astype(f32).reshape(1, M),
                           jnp.zeros((3, M), f32)], axis=0)
    coef_v[...] = tab.T

    c_x.wait()
    for j in range(S // 512):
        x_v[j * 512:(j + 1) * 512, :] = xT_v[:, j * 512:(j + 1) * 512].T
    c_wq.wait()
    for j in range(NQSTEP):
        for c in w_copies(j):
            c.start()
    c_c.start()
    c_k.start()
    c_vv.start()
    c_sk.start()
    c_q.start()
    c_wo.start()
    for j in range(M // 64):
        wq_p[:, j * 64:(j + 1) * 64, :] = pltpu.einshape("chd->hcd", wq_raw[j * 64:(j + 1) * 64])

    def qstep(j, carry):
        for c in w_copies(j):
            c.wait()
        npc = CCH // RP
        pieces = [(t, w) for t in range(npc) for w in range(2)]
        nmm = len(pieces) // HPS
        rows = S // nmm
        for hh in range(HPS):
            h = j * HPS + hh
            for r in range(nmm):
                qh = jnp.dot(x_v[r * rows:(r + 1) * rows, :], wq_p[h], preferred_element_type=f32)
                qw_v[h, r * rows:(r + 1) * rows, :] = (qh * QSCALE).astype(bf16)
                t, w = pieces.pop(0)
                src = pl.ds(pl.multiple_of(j * CCH + t * RP, RP), RP)
                dst = pl.ds(pl.multiple_of(w * C + j * CCH + t * RP, RP), RP)
                raw = wuk_raw if w == 0 else wuv_raw
                qw_v[H:2 * H, dst, :] = pltpu.einshape("chd->hcd", raw[src])
        return carry
    lax.fori_loop(0, NQSTEP, qstep, 0)

    c_c.wait()
    c_k.wait()
    c_vv.wait()
    c_sk.wait()
    c_q.wait()
    c_wo.wait()

    def head(h, carry):
        r0 = pl.multiple_of(jnp.minimum(h * CH, M - CH), CH)
        conv = _Conv(r0, qT_v, kT_v, vT_v, sk_v, coef_v, fwd_ref, inv_ref, aT_v)
        _head_body(h, c_v, qw_v, k_s, v_s, qw_v, ctx_v, conv)
        return carry
    lax.fori_loop(0, H, head, 0)

    def ostep(j, carry):
        rs = pl.ds(pl.multiple_of(j * BQ, BQ), BQ)
        bT = lax.dot_general(wo_v[0], ctx_v[0, rs, :], NT, preferred_element_type=f32)
        for h in range(1, H):
            bT = bT + lax.dot_general(wo_v[h], ctx_v[h, rs, :], NT, preferred_element_type=f32)
        full = jnp.concatenate([aT_v[:, rs], bT], axis=0)
        o_s[rs, :] = full.T.astype(bf16)
        cp(o_s.at[rs], out_h.at[rs], sem_o.at[j]).start()
        return carry
    lax.fori_loop(0, S // BQ, ostep, 0)
    for j in range(S // BQ):
        cp(o_s.at[j * BQ:(j + 1) * BQ], out_h.at[j * BQ:(j + 1) * BQ], sem_o.at[j]).wait()


@jax.jit
def pallas_concat_heads__ssm_conv_h3__compressed_kv_cla__prompt_kernel(
    A_q: jax.Array,
    A_k: jax.Array,
    A_v: jax.Array,
    A_shift_k: jax.Array,
    A_ssm_k: jax.Array,
    A_ssm_D: jax.Array,
    B_x: jax.Array,
    B_c_kv: jax.Array,
    B_w_q: jax.Array,
    B_w_uk: jax.Array,
    B_w_uv: jax.Array,
    B_w_o: jax.Array,
):
    fwd, inv = _dft_mats()
    hbm = pl.BlockSpec(memory_space=pltpu.HBM)
    vmem = pl.BlockSpec(memory_space=pltpu.VMEM)
    V = pltpu.VMEM
    out = pl.pallas_call(
        _kernel,
        out_shape=jax.ShapeDtypeStruct((S, 2 * M), bf16),
        in_specs=[hbm, hbm, hbm, vmem, hbm, vmem, hbm, hbm, hbm, hbm, hbm, hbm, vmem, vmem],
        out_specs=hbm,
        scratch_shapes=[
            V((M, S), bf16), V((M, S), bf16), V((M, S), bf16), V((M, S), bf16),
            V((M, S), bf16), V((S, M), bf16), V((S, C), bf16),
            V((M, H, D), bf16), V((H, M, D), bf16),
            V((C, H, D), bf16), V((C, H, D), bf16),
            V((2 * H, S, D), bf16), V((H, S, D), bf16),
            V((H, M, D), bf16), V((M, S), f32), V((M, 8), f32),
            V((S, D), bf16), V((S, D), bf16), V((S, 2 * M), bf16),
            pltpu.SemaphoreType.DMA((8,)),
            pltpu.SemaphoreType.DMA((2, NQSTEP)),
            pltpu.SemaphoreType.DMA((S // BQ,)),
        ],
        compiler_params=pltpu.CompilerParams(vmem_limit_bytes=120 * 1024 * 1024),
    )(A_q[0].T, A_k[0].T, A_v[0].T, A_shift_k.T, A_ssm_k, A_ssm_D, B_x[0].T, B_c_kv[0],
      B_w_q, B_w_uk, B_w_uv, jnp.swapaxes(B_w_o, 1, 2), fwd, inv)
    return out[None]
```

```python
import numpy as np
import jax
import jax.numpy as jnp
from jax import lax
import jax.experimental.pallas as pl
import jax.experimental.pallas.tpu as pltpu

f32 = jnp.float32
bf16 = jnp.bfloat16
u32 = jnp.uint32
NT = (((1,), (1,)), ((), ()))

S = 2048
M = 448
H = 16
D = 256
C = 1024
T = 128
NB = S // T
BQ = 256
CH = 32
NEG = -1e30
QSCALE = float(D ** -0.5 * np.log2(np.e))


def _pk(x):
    return pltpu.bitcast(x, u32)


def _up(x):
    return pltpu.bitcast(x, bf16)


def _dft_mats():
    n = np.arange(T)[:, None]
    f = np.arange(T)[None, :]
    th = 2 * np.pi * (f + 0.5) * n / (2 * T)
    fwd = np.concatenate([np.cos(th), -np.sin(th)], axis=1)
    n2 = (T + np.arange(T))[None, :]
    f2 = np.arange(T)[:, None]
    th2 = 2 * np.pi * (f2 + 0.5) * n2 / (2 * T)
    inv = np.concatenate([np.cos(th2), -np.sin(th2)], axis=0) / T
    return jnp.asarray(fwd, bf16), jnp.asarray(inv, bf16)


class _Conv:
    def __init__(self, r0, qT_v, kT_v, vT_v, sk_v, coef_v, fwd_ref, inv_ref, aT_v):
        self.rows = pl.ds(r0, CH)
        self.refs = (qT_v, kT_v, vT_v, sk_v, coef_v, fwd_ref, inv_ref, aT_v)
        self.ys = [[None] * (CH // 8) for _ in range(NB)]
        self.w = {}
        self.yt = [None] * (CH // 8)

    def prep(self):
        qT_v, kT_v, vT_v, sk_v, coef_v, fwd_ref, inv_ref, aT_v = self.refs
        rows = self.rows
        k = kT_v[rows, :].astype(f32)
        coef = coef_v[rows, :]
        lane = lax.broadcasted_iota(jnp.int32, (CH, S), 1)
        ks = k * coef[:, 0:1]
        for j in range(1, 4):
            kj = jnp.where(lane >= j, pltpu.roll(k, j, axis=1), 0.0)
            ks = ks + kj * coef[:, j:j + 1]
        self.u = (ks * vT_v[rows, :].astype(f32)).astype(bf16)
        self.dcol = coef[:, 4:5]

    def fwd(self):
        qT_v, kT_v, vT_v, sk_v, coef_v, fwd_ref, inv_ref, aT_v = self.refs
        u = self.u
        sk = sk_v[self.rows, :]
        lhs = jnp.concatenate(
            [u[:, a * T:(a + 1) * T] for a in range(NB)]
            + [sk[:, a * T:(a + 1) * T] for a in range(NB)], axis=0)
        self.x = jnp.dot(lhs, fwd_ref[...], preferred_element_type=f32)

    def _blk(self, g, a, part, base):
        r = base + a * CH + g * 8
        return self.x[r:r + 8, part * T:(part + 1) * T]

    def mac(self, g, alist):
        if g not in self.w:
            flane = lax.broadcasted_iota(jnp.int32, (8, T), 1)
            sgn = jnp.where((flane & 1) == 0, 1.0, -1.0).astype(f32)
            kr = [self._blk(g, a, 0, NB * CH) for a in range(NB)]
            ki = [self._blk(g, a, 1, NB * CH) for a in range(NB)]
            wr = [sgn * ki[0]] + [kr[a - 1] + sgn * ki[a] for a in range(1, NB)]
            wi = [-(sgn * kr[0])] + [ki[a - 1] - sgn * kr[a] for a in range(1, NB)]
            self.w[g] = (wr, wi)
        wr, wi = self.w[g]
        ur = [self._blk(g, a, 0, 0) for a in range(NB)]
        ui = [self._blk(g, a, 1, 0) for a in range(NB)]
        for a in alist:
            yr = wr[0] * ur[a] - wi[0] * ui[a]
            yi = wr[0] * ui[a] + wi[0] * ur[a]
            for dl in range(1, a + 1):
                yr = yr + (wr[dl] * ur[a - dl] - wi[dl] * ui[a - dl])
                yi = yi + (wr[dl] * ui[a - dl] + wi[dl] * ur[a - dl])
            self.ys[a][g] = jnp.concatenate([yr, yi], axis=1)

    def inv(self, g):
        qT_v, inv_ref, aT_v = self.refs[0], self.refs[6], self.refs[7]
        yf = jnp.concatenate([self.ys[a][g] for a in range(NB)], axis=0)
        y = jnp.dot(yf.astype(bf16), inv_ref[...], preferred_element_type=f32)
        self.yt[g] = jnp.concatenate([y[a * 8:(a + 1) * 8, :] for a in range(NB)], axis=1)

    def gate(self):
        qT_v, aT_v = self.refs[0], self.refs[7]
        y = jnp.concatenate(self.yt, axis=0)
        aT_v[self.rows, :] = qT_v[self.rows, :].astype(f32) * (y + self.u.astype(f32) * self.dcol)


HB = BQ // 2


def _tiles(x):
    return [x[:, t * 128:(t + 1) * 128] for t in range(x.shape[1] // 128)]


def _fold(op, xs):
    r = xs[0]
    for x in xs[1:]:
        r = op(r, x)
    return r


class _QBlock:
    def __init__(self, h, i, q_v, k_s, v_s, ctx_v):
        self.h, self.i = h, i
        self.q_v, self.k_s, self.v_s, self.ctx_v = q_v, k_s, v_s, ctx_v
        self.lo = i * BQ
        end = self.lo + HB
        self.chunks = [(a, min(a + KCH, end)) for a in range(0, end, KCH)]
        self.s = [None] * len(self.chunks)
        self.p = [None] * len(self.chunks)
        self.mrun = None
        self.lrun = None
        self.acc = None

    def qk(self, c):
        lo = self.lo
        a, b = self.chunks[c]
        q = _up(self.q_v[self.h, lo // 2:(lo + BQ) // 2, :])
        s = lax.dot_general(q, _up(self.k_s[a // 2:b // 2, :]), NT, preferred_element_type=f32)
        ts = _tiles(s)
        if c == len(self.chunks) - 1:
            row = lax.broadcasted_iota(jnp.int32, (BQ, 128), 0)
            col = lax.broadcasted_iota(jnp.int32, (BQ, 128), 1)
            ts[-1] = jnp.where(col <= row, ts[-1], NEG)
            sc = lax.dot_general(q[HB:, :], _up(self.k_s[b // 2:(b + HB) // 2, :]), NT, preferred_element_type=f32)
            row = lax.broadcasted_iota(jnp.int32, (HB, 128), 0)
            col = lax.broadcasted_iota(jnp.int32, (HB, 128), 1)
            self.sc = jnp.where(col <= row, sc, NEG)
        self.s[c] = ts
        m = _fold(jnp.maximum, ts)
        self.mrun = m if self.mrun is None else jnp.maximum(self.mrun, m)

    def stats(self):
        mr = jnp.concatenate([self.mrun[:HB], jnp.maximum(self.mrun[HB:], self.sc)], axis=0)
        m = jnp.max(mr, axis=1, keepdims=True)
        l = _fold(jnp.add, [jnp.exp2(t - m) for ts in self.s for t in ts])
        l = jnp.concatenate([l[:HB], l[HB:] + jnp.exp2(self.sc - m[HB:])], axis=0)
        self.off = m + jnp.log2(jnp.sum(l, axis=1, keepdims=True))

    def pv(self, c):
        a, b = self.chunks[c]
        p = jnp.concatenate([jnp.exp2(t - self.off) for t in self.s[c]], axis=1).astype(bf16)
        r = jnp.dot(p, _up(self.v_s[a // 2:b // 2, :]), preferred_element_type=f32)
        self.acc = r if self.acc is None else self.acc + r
        if c == len(self.chunks) - 1:
            pc = jnp.exp2(self.sc - self.off[HB:]).astype(bf16)
            rc = jnp.dot(pc, _up(self.v_s[b // 2:(b + HB) // 2, :]), preferred_element_type=f32)
            self.acc = jnp.concatenate([self.acc[:HB], self.acc[HB:] + rc], axis=0)

    def finish(self):
        self.ctx_v[self.h, self.lo // 2:(self.lo + BQ) // 2, :] = _pk(self.acc.astype(bf16))


KCH = 512


def _head_body(h, c_v, wkv_p, k_s, v_s, q_v, ctx_v, conv):
    nq = S // BQ

    def proj(j, half):
        dst = k_s if half == 0 else v_s
        r = jnp.dot(_up(c_v[j * HB:(j + 1) * HB, :]), _up(wkv_p[H + h, half * C // 2:(half + 1) * C // 2, :]),
                    preferred_element_type=f32)
        dst[j * HB:(j + 1) * HB, :] = _pk(r.astype(bf16))

    blocks = [_QBlock(h, i, q_v, k_s, v_s, ctx_v) for i in range(nq)]
    proj(0, 0)
    conv.prep()
    proj(0, 1)
    conv.fwd()
    proj(1, 0)
    for c in range(len(blocks[0].chunks)):
        blocks[0].qk(c)
    proj(1, 1)
    for i in range(nq):
        cur = blocks[i]
        nxt = blocks[i + 1] if i + 1 < nq else None
        if nxt:
            for c in range(len(nxt.chunks)):
                nxt.qk(c)
        if i + 2 < nq:
            proj(i + 2, 0)
        cur.stats()
        for c in range(len(cur.chunks)):
            cur.pv(c)
        cur.finish()
        if i + 2 < nq:
            proj(i + 2, 1)
        if i < CH // 8:
            conv.mac(i, list(range(NB)))
            conv.inv(i)
        if i == CH // 8:
            conv.gate()


NQSTEP = 8
HPS = H // NQSTEP
RP = 16
CCH = C // NQSTEP


def _kernel(qT_h, kT_h, vT_h, shk_ref, sk_h, d_ref, xT_h, c_h, wq_h, wuk_h, wuv_h, woT_h,
            fwd_ref, inv_ref, out_h,
            qT_v, kT_v, vT_v, sk_v, xT_v, x_v, c_v, c_p, wq_raw, wq_p, wuk_raw, wuv_raw,
            qw_v, ctx_v, wo_v, aT_v, coef_v, k_s, v_s, o_s,
            sem, sem_w, sem_o):
    cp = pltpu.make_async_copy
    c_x = cp(xT_h, xT_v, sem.at[0])
    c_wq = cp(wq_h, wq_raw, sem.at[1])
    c_c = cp(c_h, c_v, sem.at[2])
    c_k = cp(kT_h, kT_v, sem.at[3])
    c_vv = cp(vT_h, vT_v, sem.at[4])
    c_sk = cp(sk_h, sk_v, sem.at[5])
    c_q = cp(qT_h, qT_v, sem.at[6])
    c_wo = cp(woT_h, wo_v, sem.at[7])

    def w_copies(j):
        rs = pl.ds(pl.multiple_of(j * CCH, CCH), CCH) if not isinstance(j, int) else pl.ds(j * CCH, CCH)
        return (cp(wuk_h.at[rs], wuk_raw.at[rs], sem_w.at[0, j]),
                cp(wuv_h.at[rs], wuv_raw.at[rs], sem_w.at[1, j]))

    c_x.start()
    c_wq.start()

    tab = jnp.concatenate([shk_ref[...].astype(f32), d_ref[...].astype(f32).reshape(1, M),
                           jnp.zeros((3, M), f32)], axis=0)
    coef_v[...] = tab.T

    c_x.wait()
    for j in range(S // 512):
        x_v[j * 256:(j + 1) * 256, :] = _pk(xT_v[:, j * 512:(j + 1) * 512].T)
    c_wq.wait()
    for j in range(NQSTEP):
        for c in w_copies(j):
            c.start()
    c_c.start()
    c_k.start()
    c_vv.start()
    c_sk.start()
    c_q.start()
    c_wo.start()
    for j in range(M // 64):
        wq_p[:, j * 32:(j + 1) * 32, :] = _pk(pltpu.einshape("chd->hcd", wq_raw[j * 64:(j + 1) * 64]))

    def qstep(j, carry):
        for c in w_copies(j):
            c.wait()
        npc = CCH // RP
        pieces = [(t, w) for t in range(npc) for w in range(2)]
        nmm = len(pieces) // HPS
        rows = S // nmm
        for hh in range(HPS):
            h = j * HPS + hh
            for r in range(nmm):
                qh = jnp.dot(_up(x_v[r * rows // 2:(r + 1) * rows // 2, :]), _up(wq_p[h]),
                             preferred_element_type=f32)
                qw_v[h, r * rows // 2:(r + 1) * rows // 2, :] = _pk((qh * QSCALE).astype(bf16))
                t, w = pieces.pop(0)
                src = pl.ds(pl.multiple_of(j * CCH + t * RP, RP), RP)
                dst = pl.ds(pl.multiple_of((w * C + t * RP) // 2 + j * (CCH // 2), RP // 2), RP // 2)
                raw = wuk_raw if w == 0 else wuv_raw
                qw_v[H:2 * H, dst, :] = _pk(pltpu.einshape("chd->hcd", raw[src]))
        return carry
    lax.fori_loop(0, NQSTEP, qstep, 0)

    c_c.wait()
    for j in range(S // 256):
        c_p[j * 128:(j + 1) * 128, :] = _pk(c_v[j * 256:(j + 1) * 256, :])
    c_k.wait()
    c_vv.wait()
    c_sk.wait()
    c_q.wait()
    c_wo.wait()

    def head(h, carry):
        r0 = pl.multiple_of(jnp.minimum(h * CH, M - CH), CH)
        conv = _Conv(r0, qT_v, kT_v, vT_v, sk_v, coef_v, fwd_ref, inv_ref, aT_v)
        _head_body(h, c_p, qw_v, k_s, v_s, qw_v, ctx_v, conv)
        return carry
    lax.fori_loop(0, H, head, 0)

    def ostep(j, carry):
        rs = pl.ds(pl.multiple_of(j * BQ, BQ), BQ)
        rp = pl.ds(pl.multiple_of(j * HB, HB), HB)
        bT = lax.dot_general(wo_v[0], _up(ctx_v[0, rp, :]), NT, preferred_element_type=f32)
        for h in range(1, H):
            bT = bT + lax.dot_general(wo_v[h], _up(ctx_v[h, rp, :]), NT, preferred_element_type=f32)
        full = jnp.concatenate([aT_v[:, rs], bT], axis=0)
        o_s[rs, :] = full.T.astype(bf16)
        cp(o_s.at[rs], out_h.at[rs], sem_o.at[j]).start()
        return carry
    lax.fori_loop(0, S // BQ, ostep, 0)
    for j in range(S // BQ):
        cp(o_s.at[j * BQ:(j + 1) * BQ], out_h.at[j * BQ:(j + 1) * BQ], sem_o.at[j]).wait()


@jax.jit
def pallas_concat_heads__ssm_conv_h3__compressed_kv_cla__prompt_kernel(
    A_q: jax.Array,
    A_k: jax.Array,
    A_v: jax.Array,
    A_shift_k: jax.Array,
    A_ssm_k: jax.Array,
    A_ssm_D: jax.Array,
    B_x: jax.Array,
    B_c_kv: jax.Array,
    B_w_q: jax.Array,
    B_w_uk: jax.Array,
    B_w_uv: jax.Array,
    B_w_o: jax.Array,
):
    fwd, inv = _dft_mats()
    hbm = pl.BlockSpec(memory_space=pltpu.HBM)
    vmem = pl.BlockSpec(memory_space=pltpu.VMEM)
    V = pltpu.VMEM
    out = pl.pallas_call(
        _kernel,
        out_shape=jax.ShapeDtypeStruct((S, 2 * M), bf16),
        in_specs=[hbm, hbm, hbm, vmem, hbm, vmem, hbm, hbm, hbm, hbm, hbm, hbm, vmem, vmem],
        out_specs=hbm,
        scratch_shapes=[
            V((M, S), bf16), V((M, S), bf16), V((M, S), bf16), V((M, S), bf16),
            V((M, S), bf16), V((S // 2, M), u32), V((S, C), bf16), V((S // 2, C), u32),
            V((M, H, D), bf16), V((H, M // 2, D), u32),
            V((C, H, D), bf16), V((C, H, D), bf16),
            V((2 * H, S // 2, D), u32), V((H, S // 2, D), u32),
            V((H, M, D), bf16), V((M, S), f32), V((M, 8), f32),
            V((S // 2, D), u32), V((S // 2, D), u32), V((S, 2 * M), bf16),
            pltpu.SemaphoreType.DMA((8,)),
            pltpu.SemaphoreType.DMA((2, NQSTEP)),
            pltpu.SemaphoreType.DMA((S // BQ,)),
        ],
        compiler_params=pltpu.CompilerParams(vmem_limit_bytes=120 * 1024 * 1024),
    )(A_q[0].T, A_k[0].T, A_v[0].T, A_shift_k.T, A_ssm_k, A_ssm_D, B_x[0].T, B_c_kv[0],
      B_w_q, B_w_uk, B_w_uv, jnp.swapaxes(B_w_o, 1, 2), fwd, inv)
    return out[None]
```

```python
import numpy as np
import jax
import jax.numpy as jnp
from jax import lax
import jax.experimental.pallas as pl
import jax.experimental.pallas.tpu as pltpu

f32 = jnp.float32
bf16 = jnp.bfloat16
u32 = jnp.uint32
NT = (((1,), (1,)), ((), ()))

S = 2048
M = 448
H = 16
D = 256
C = 1024
T = 128
NB = S // T
BQ = 256
CH = 32
NEG = -1e30
CFG = dict(KCH_QK=512, KCH_PV=512, ORDER='d', CV0=2, QSPLIT=2, OST=8, MLAG=2, TIE0=3, SER=32, SER0=3)
QSCALE = float(D ** -0.5 * np.log2(np.e))


def _pk(x):
    return pltpu.bitcast(x, u32)


def _up(x):
    return pltpu.bitcast(x, bf16)


def _opq(x, h):
    return x ^ lax.shift_right_logical(h, 8).astype(u32)


def _tie(x, dep, h):
    d = pltpu.bitcast(dep, u32)
    z = _fold(jnp.bitwise_or, [d[r * 8:(r + 1) * 8, :] for r in range(d.shape[0] // 8)])
    z = z & lax.shift_right_logical(h, 8).astype(u32)
    top = jnp.concatenate([x[0:8, 0:128] ^ z, x[0:8, 128:]], axis=1)
    return jnp.concatenate([top, x[8:]], axis=0)


def _dft_mats():
    n = np.arange(T)[:, None]
    f = np.arange(T)[None, :]
    th = 2 * np.pi * (f + 0.5) * n / (2 * T)
    fwd = np.concatenate([np.cos(th), -np.sin(th)], axis=1)
    n2 = (T + np.arange(T))[None, :]
    f2 = np.arange(T)[:, None]
    th2 = 2 * np.pi * (f2 + 0.5) * n2 / (2 * T)
    inv = np.concatenate([np.cos(th2), -np.sin(th2)], axis=0) / T
    return jnp.asarray(fwd, bf16), jnp.asarray(inv, bf16)


class _Conv:
    def __init__(self, r0, qT_v, kT_v, vT_v, sk_v, coef_v, fwd_ref, inv_ref, aT_v):
        self.rows = pl.ds(r0, CH)
        self.refs = (qT_v, kT_v, vT_v, sk_v, coef_v, fwd_ref, inv_ref, aT_v)
        self.ys = [[None] * (CH // 8) for _ in range(NB)]
        self.w = {}
        self.yt = [None] * (CH // 8)

    def prep(self):
        qT_v, kT_v, vT_v, sk_v, coef_v, fwd_ref, inv_ref, aT_v = self.refs
        rows = self.rows
        k = kT_v[rows, :].astype(f32)
        coef = coef_v[rows, :]
        lane = lax.broadcasted_iota(jnp.int32, (CH, S), 1)
        ks = k * coef[:, 0:1]
        for j in range(1, 4):
            kj = jnp.where(lane >= j, pltpu.roll(k, j, axis=1), 0.0)
            ks = ks + kj * coef[:, j:j + 1]
        self.u = (ks * vT_v[rows, :].astype(f32)).astype(bf16)
        self.dcol = coef[:, 4:5]

    def fwd(self):
        qT_v, kT_v, vT_v, sk_v, coef_v, fwd_ref, inv_ref, aT_v = self.refs
        u = self.u
        sk = sk_v[self.rows, :]
        lhs = jnp.concatenate(
            [u[:, a * T:(a + 1) * T] for a in range(NB)]
            + [sk[:, a * T:(a + 1) * T] for a in range(NB)], axis=0)
        self.x = jnp.dot(lhs, fwd_ref[...], preferred_element_type=f32)

    def _blk(self, g, a, part, base):
        r = base + a * CH + g * 8
        return self.x[r:r + 8, part * T:(part + 1) * T]

    def mac(self, g, alist):
        if g not in self.w:
            flane = lax.broadcasted_iota(jnp.int32, (8, T), 1)
            sgn = jnp.where((flane & 1) == 0, 1.0, -1.0).astype(f32)
            kr = [self._blk(g, a, 0, NB * CH) for a in range(NB)]
            ki = [self._blk(g, a, 1, NB * CH) for a in range(NB)]
            wr = [sgn * ki[0]] + [kr[a - 1] + sgn * ki[a] for a in range(1, NB)]
            wi = [-(sgn * kr[0])] + [ki[a - 1] - sgn * kr[a] for a in range(1, NB)]
            self.w[g] = (wr, wi)
        wr, wi = self.w[g]
        ur = [self._blk(g, a, 0, 0) for a in range(NB)]
        ui = [self._blk(g, a, 1, 0) for a in range(NB)]
        for a in alist:
            yr = wr[0] * ur[a] - wi[0] * ui[a]
            yi = wr[0] * ui[a] + wi[0] * ur[a]
            for dl in range(1, a + 1):
                yr = yr + (wr[dl] * ur[a - dl] - wi[dl] * ui[a - dl])
                yi = yi + (wr[dl] * ui[a - dl] + wi[dl] * ur[a - dl])
            self.ys[a][g] = jnp.concatenate([yr, yi], axis=1)

    def inv(self, g):
        qT_v, inv_ref, aT_v = self.refs[0], self.refs[6], self.refs[7]
        yf = jnp.concatenate([self.ys[a][g] for a in range(NB)], axis=0)
        y = jnp.dot(yf.astype(bf16), inv_ref[...], preferred_element_type=f32)
        self.yt[g] = jnp.concatenate([y[a * 8:(a + 1) * 8, :] for a in range(NB)], axis=1)

    def gate(self):
        qT_v, aT_v = self.refs[0], self.refs[7]
        y = jnp.concatenate(self.yt, axis=0)
        aT_v[self.rows, :] = qT_v[self.rows, :].astype(f32) * (y + self.u.astype(f32) * self.dcol)


HB = BQ // 2


def _tiles(x):
    return [x[:, t * 128:(t + 1) * 128] for t in range(x.shape[1] // 128)]


def _fold(op, xs):
    r = xs[0]
    for x in xs[1:]:
        r = op(r, x)
    return r


class _QBlock:
    def __init__(self, h, i, q_v, k_s, v_s, ctx_v):
        self.h, self.i = h, i
        self.q_v, self.k_s, self.v_s, self.ctx_v = q_v, k_s, v_s, ctx_v
        self.lo = i * BQ
        self.end = self.lo + HB
        self.t = []

    def qk(self):
        lo, end = self.lo, self.end
        KCH = CFG['KCH_QK']
        q = _up(_opq(_pk(self.q_v[self.h, lo:lo + BQ, :]), self.h))
        LAG = CFG['MLAG']
        self.mrun, self.nm = None, 0
        for ci, a in enumerate(range(0, end, KCH)):
            b = min(a + KCH, end)
            kk = self.k_s[a // 2:b // 2, :]
            if LAG and ci >= LAG and self.i >= CFG['TIE0']:
                upto = (ci - LAG + 1) * KCH // 128
                self.mrun = _fold(jnp.maximum, ([self.mrun] if self.nm else []) + self.t[self.nm:upto])
                self.nm = upto
                kk = _tie(kk, self.mrun, self.h)
            s = lax.dot_general(q, _up(kk), NT, preferred_element_type=f32)
            self.t += _tiles(s)
        row = lax.broadcasted_iota(jnp.int32, (BQ, 128), 0)
        col = lax.broadcasted_iota(jnp.int32, (BQ, 128), 1)
        self.t[-1] = jnp.where(col <= row, self.t[-1], NEG)
        sc = lax.dot_general(q[HB:, :], _up(self.k_s[end // 2:(end + HB) // 2, :]), NT,
                             preferred_element_type=f32)
        row = lax.broadcasted_iota(jnp.int32, (HB, 128), 0)
        col = lax.broadcasted_iota(jnp.int32, (HB, 128), 1)
        self.sc = jnp.where(col <= row, sc, NEG)

    def stats(self):
        mrun = _fold(jnp.maximum, ([self.mrun] if self.nm else []) + self.t[self.nm:])
        mr = jnp.concatenate([mrun[:HB], jnp.maximum(mrun[HB:], self.sc)], axis=0)
        m = jnp.max(mr, axis=1, keepdims=True)
        R = CFG['SER']
        if R and self.i >= CFG['SER0']:
            zero = lax.shift_right_logical(self.h, 8).astype(u32)
            mb = jnp.broadcast_to(m, (BQ, 128))
            ls = []
            for g in range(BQ // R):
                mg = mb[g * R:(g + 1) * R]
                if ls:
                    z = pltpu.bitcast(pltpu.bitcast(ls[-1], u32) & zero, f32)
                    mg = mg + z
                ts = [t[g * R:(g + 1) * R] for t in self.t]
                if g * R >= HB:
                    ts.append(self.sc[g * R - HB:(g + 1) * R - HB])
                ls.append(_fold(jnp.add, [jnp.exp2(t - mg) for t in ts]))
            l = jnp.concatenate(ls, axis=0)
        else:
            l = _fold(jnp.add, [jnp.exp2(t - m) for t in self.t])
            l = jnp.concatenate([l[:HB], l[HB:] + jnp.exp2(self.sc - m[HB:])], axis=0)
        self.off = m + jnp.log2(jnp.sum(l, axis=1, keepdims=True))

    def pv(self):
        end = self.end
        KCH = CFG['KCH_PV']
        acc = None
        for a in range(0, end, KCH):
            b = min(a + KCH, end)
            p = jnp.concatenate([jnp.exp2(t - self.off) for t in self.t[a // 128:b // 128]],
                                axis=1).astype(bf16)
            r = jnp.dot(p, _up(self.v_s[a // 2:b // 2, :]), preferred_element_type=f32)
            acc = r if acc is None else acc + r
        pc = jnp.exp2(self.sc - self.off[HB:]).astype(bf16)
        rc = jnp.dot(pc, _up(self.v_s[end // 2:(end + HB) // 2, :]), preferred_element_type=f32)
        acc = jnp.concatenate([acc[:HB], acc[HB:] + rc], axis=0)
        self.ctx_v[self.h, self.lo // 2:(self.lo + BQ) // 2, :] = _pk(acc.astype(bf16))


def _head_body(h, c_p, qw_v, k_s, v_s, ctx_v, conv):
    nq = S // BQ
    w = {}

    def proj(j, half):
        dst = k_s if half == 0 else v_s
        if half not in w:
            w[half] = _up(_opq(_pk(qw_v[H + h, half * C:(half + 1) * C, :]), h))
        r = jnp.dot(_up(c_p[j * HB:(j + 1) * HB, :]), w[half], preferred_element_type=f32)
        dst[j * HB:(j + 1) * HB, :] = _pk(r.astype(bf16))

    def convpiece(i):
        if 0 <= i < CH // 8:
            conv.mac(i, list(range(NB)))
            conv.inv(i)
        if i == CH // 8:
            conv.gate()

    B = [_QBlock(h, i, qw_v, k_s, v_s, ctx_v) for i in range(nq)]
    proj(0, 0)
    conv.prep()
    proj(1, 0)
    conv.fwd()
    B[0].qk()
    proj(0, 1)
    for i in range(nq):
        if i + 1 < nq:
            B[i + 1].qk()
            proj(i + 1, 1)
        B[i].stats()
        B[i].pv()
        if i + 2 < nq:
            proj(i + 2, 0)
        convpiece(i - CFG['CV0'])


NR = 4
XR = S // NR
HH = H // 2
RP = 16
QR = M // NR
WR = C // NR


def _kernel(qT_h, kT_h, vT_h, shk_h, sk_h, d_h, xT_h, c_h, wq_h, wuk_h, wuv_h, woT_h,
            fwd_h, inv_h, out_h,
            qT_v, kT_v, vT_v, sk_v, xT_v, x_v, c_v, c_p, wq_raw, wq0_p, wq1_p, wuk_raw, wuv_raw,
            qw_v, ctx_v, wo_v, aT_v, coef_v, k_s, v_s, o_s, shk_v, d_v, fwd_v, inv_v,
            sem, sem_q, sem_w, sem_o):
    cp = pltpu.make_async_copy
    c_x = cp(xT_h, xT_v, sem.at[0])
    c_c = cp(c_h, c_v, sem.at[1])
    late = [cp(kT_h, kT_v, sem.at[2]), cp(vT_h, vT_v, sem.at[3]), cp(sk_h, sk_v, sem.at[4]),
            cp(qT_h, qT_v, sem.at[5])]
    c_wo = cp(woT_h, wo_v, sem.at[6])
    tiny = [cp(shk_h, shk_v, sem.at[7]), cp(d_h, d_v, sem.at[8]), cp(fwd_h, fwd_v, sem.at[9]),
            cp(inv_h, inv_v, sem.at[10])]

    def rows(j, n):
        return pl.ds(j * n, n) if isinstance(j, int) else pl.ds(pl.multiple_of(j * n, n), n)

    def wq_copy(g, j):
        return cp(wq_h.at[rows(j, QR), g * HH:(g + 1) * HH, :], wq_raw.at[g, rows(j, QR)], sem_q.at[g, j])

    def w_copies(j):
        return (cp(wuk_h.at[rows(j, WR)], wuk_raw.at[rows(j, WR)], sem_w.at[0, j]),
                cp(wuv_h.at[rows(j, WR)], wuv_raw.at[rows(j, WR)], sem_w.at[1, j]))

    def start_seq(fn):
        def body(j, carry):
            for c in fn(j):
                c.start()
            return carry
        lax.fori_loop(0, NR, body, 0)

    for c in tiny:
        c.start()
    c_x.start()
    start_seq(lambda j: (wq_copy(0, j),))
    start_seq(lambda j: (wq_copy(1, j),))
    c_c.start()
    start_seq(w_copies)
    for c in late:
        c.start()
    c_wo.start()

    for c in tiny:
        c.wait()
    tab = jnp.concatenate([shk_v[...].astype(f32), d_v[...].astype(f32).reshape(1, M),
                           jnp.zeros((3, M), f32)], axis=0)
    coef_v[...] = tab.T

    c_x.wait()
    for j in range(S // 512):
        x_v[j * 256:(j + 1) * 256, :] = _pk(xT_v[:, j * 512:(j + 1) * 512].T)
    for j in range(NR):
        wq_copy(0, j).wait()
        for t in range(QR // RP):
            r = j * QR + t * RP
            wq0_p[:, r:r + RP, :] = pltpu.einshape("chd->hcd", wq_raw[0, r:r + RP])

    def qproj_step(r, g, wq, pieces):
        QS = CFG['QSPLIT']
        n = XR // QS
        x = [_up(_opq(x_v[pl.ds(pl.multiple_of(r * (XR // 2) + s * (n // 2), n // 2), n // 2), :], r))
             for s in range(QS)]
        slots = HH * QS
        npc = len(pieces)
        done = 0
        deps = []
        for k in range(slots):
            hh, s = k // QS, k % QS
            qh = jnp.dot(x[s], wq(hh), preferred_element_type=f32)
            if deps:
                z = _fold(jnp.bitwise_or, [d[..., t * 8:(t + 1) * 8, u * 128:(u + 1) * 128].reshape(-1, 8, 128)[v]
                                           for d in deps for t in range(d.shape[-2] // 8)
                                           for u in range(d.shape[-1] // 128)
                                           for v in range(d.size // (d.shape[-1] * d.shape[-2]))])
                z = pltpu.bitcast(z & lax.shift_right_logical(r, 8).astype(u32), f32)
                top = jnp.concatenate([qh[0:8, 0:128] + z, qh[0:8, 128:]], axis=1)
                qh = jnp.concatenate([top, qh[8:]], axis=0)
                deps = []
            qw_v[g * HH + hh, pl.ds(pl.multiple_of(r * XR + s * n, n), n), :] = (qh * QSCALE).astype(bf16)
            want = min(npc, -(-(k + 1) * npc // (slots - 1)))
            while done < want:
                d = pieces[done]()
                if d is not None:
                    deps.append(d)
                done += 1

    def step_a(r, carry):
        wq_copy(1, r).wait()

        def piece(t):
            def run():
                rs = pl.ds(pl.multiple_of(r * QR + t * RP, RP), RP)
                rd = pl.ds(pl.multiple_of(r * (QR // 2) + t * (RP // 2), RP // 2), RP // 2)
                val = _pk(pltpu.einshape("chd->hcd", wq_raw[1, rs]))
                wq1_p[:, rd, :] = val
                return val
            return run
        qproj_step(r, 0, lambda hh: wq0_p[hh], [piece(t) for t in range(QR // RP)])
        return carry
    lax.fori_loop(0, NR, step_a, 0)

    c_c.wait()

    def step_b(r, carry):
        for c in w_copies(r):
            c.wait()

        def piece(t, w):
            def run():
                src = pl.ds(pl.multiple_of(r * WR + t * RP, RP), RP)
                dst = pl.ds(pl.multiple_of(w * C + r * WR + t * RP, RP), RP)
                raw = wuk_raw if w == 0 else wuv_raw
                qw_v[H:2 * H, dst, :] = pltpu.einshape("chd->hcd", raw[src])
                if w == 0 and t % 2 == 0:
                    n = XR // (WR // RP // 2)
                    o = r * XR + (t // 2) * n
                    val = _pk(c_v[pl.ds(pl.multiple_of(o, n), n), :])
                    c_p[pl.ds(pl.multiple_of(o // 2, n // 2), n // 2), :] = val
                    return val
            return run
        qproj_step(r, 1, lambda hh: _up(wq1_p[hh]), [piece(t, w) for t in range(WR // RP) for w in range(2)])
        return carry
    lax.fori_loop(0, NR, step_b, 0)

    for c in late:
        c.wait()

    def head(h, carry):
        r0 = pl.multiple_of(jnp.minimum(h * CH, M - CH), CH)
        conv = _Conv(r0, qT_v, kT_v, vT_v, sk_v, coef_v, fwd_v, inv_v, aT_v)
        _head_body(h, c_p, qw_v, k_s, v_s, ctx_v, conv)
        return carry
    lax.fori_loop(0, H, head, 0)

    c_wo.wait()
    OST = CFG['OST']
    OR = S // OST

    def ostep(j, carry):
        rs = pl.ds(pl.multiple_of(j * OR, OR), OR)
        rp = pl.ds(pl.multiple_of(j * (OR // 2), OR // 2), OR // 2)
        bT = lax.dot_general(wo_v[0], _up(ctx_v[0, rp, :]), NT, preferred_element_type=f32)
        for h in range(1, H):
            bT = bT + lax.dot_general(wo_v[h], _up(ctx_v[h, rp, :]), NT, preferred_element_type=f32)
        full = jnp.concatenate([aT_v[:, rs], bT], axis=0)
        o_s[rs, :] = full.T.astype(bf16)
        cp(o_s.at[rs], out_h.at[rs], sem_o.at[j]).start()
        return carry
    lax.fori_loop(0, OST, ostep, 0)
    for j in range(OST):
        cp(o_s.at[j * OR:(j + 1) * OR], out_h.at[j * OR:(j + 1) * OR], sem_o.at[j]).wait()


@jax.jit
def pallas_concat_heads__ssm_conv_h3__compressed_kv_cla__prompt_kernel(
    A_q: jax.Array,
    A_k: jax.Array,
    A_v: jax.Array,
    A_shift_k: jax.Array,
    A_ssm_k: jax.Array,
    A_ssm_D: jax.Array,
    B_x: jax.Array,
    B_c_kv: jax.Array,
    B_w_q: jax.Array,
    B_w_uk: jax.Array,
    B_w_uv: jax.Array,
    B_w_o: jax.Array,
):
    fwd, inv = _dft_mats()
    hbm = pl.BlockSpec(memory_space=pltpu.HBM)
    V = pltpu.VMEM
    out = pl.pallas_call(
        _kernel,
        out_shape=jax.ShapeDtypeStruct((S, 2 * M), bf16),
        in_specs=[hbm] * 14,
        out_specs=hbm,
        scratch_shapes=[
            V((M, S), bf16), V((M, S), bf16), V((M, S), bf16), V((M, S), bf16),
            V((M, S), bf16), V((S // 2, M), u32),
            V((S, C), bf16), V((S // 2, C), u32),
            V((2, M, HH, D), bf16), V((HH, M, D), bf16), V((HH, M // 2, D), u32),
            V((C, H, D), bf16), V((C, H, D), bf16),
            V((2 * H, S, D), bf16), V((H, S // 2, D), u32),
            V((H, M, D), bf16), V((M, S), f32), V((M, 8), f32),
            V((S // 2, D), u32), V((S // 2, D), u32), V((S, 2 * M), bf16),
            V((4, M), bf16), V((M,), bf16), V((T, 2 * T), bf16), V((2 * T, T), bf16),
            pltpu.SemaphoreType.DMA((11,)),
            pltpu.SemaphoreType.DMA((2, NR)),
            pltpu.SemaphoreType.DMA((2, NR)),
            pltpu.SemaphoreType.DMA((8,)),
        ],
        compiler_params=pltpu.CompilerParams(vmem_limit_bytes=120 * 1024 * 1024),
    )(A_q[0].T, A_k[0].T, A_v[0].T, A_shift_k.T, A_ssm_k, A_ssm_D, B_x[0].T, B_c_kv[0],
      B_w_q, B_w_uk, B_w_uv, jnp.swapaxes(B_w_o, 1, 2), fwd, inv)
    return out[None]
```

```python
import numpy as np
import jax
import jax.numpy as jnp
from jax import lax
import jax.experimental.pallas as pl
import jax.experimental.pallas.tpu as pltpu

f32 = jnp.float32
bf16 = jnp.bfloat16
u32 = jnp.uint32
NT = (((1,), (1,)), ((), ()))

S = 2048
M = 448
H = 16
D = 256
C = 1024
T = 128
NB = S // T
BQ = 256
CH = 24
CB = M - H * CH
NEG = -1e30
CFG = dict(KCH_QK=512, KCH_PV=512, OST=4, OSUB=2, OTIE=0, SER=32, SER0=5, PSPLIT=1, N1=7, N2=3,
           CPLAN=[(1, 5, 2, 5, 3, 4), (3, 5, 4, 5, 5, 4), (4, 5, 5, 5, 6, 4)],
           APLAN=(0, 3, 4))
QSCALE = float(D ** -0.5 * np.log2(np.e))


def _tiles(x):
    return [x[:, t * 128:(t + 1) * 128] for t in range(x.shape[1] // 128)]


def _fold(op, xs):
    r = xs[0]
    for x in xs[1:]:
        r = op(r, x)
    return r


def _pk(x):
    return pltpu.bitcast(x, u32)


def _up(x):
    return pltpu.bitcast(x, bf16)


def _opq(x, h):
    return x ^ lax.shift_right_logical(h, 8).astype(u32)


def _tie(x, dep, h):
    d = dep if dep.dtype == u32 else pltpu.bitcast(dep, u32)
    z = _fold(jnp.bitwise_or, [d[r * 8:(r + 1) * 8, :] for r in range(d.shape[0] // 8)])
    z = z & lax.shift_right_logical(h, 8).astype(u32)
    top = jnp.concatenate([x[0:8, 0:128] ^ z, x[0:8, 128:]], axis=1)
    return jnp.concatenate([top, x[8:]], axis=0)


def _dft_mats():
    n = np.arange(T)[:, None]
    f = np.arange(T)[None, :]
    th = 2 * np.pi * (f + 0.5) * n / (2 * T)
    fwd = np.concatenate([np.cos(th), -np.sin(th)], axis=1)
    n2 = (T + np.arange(T))[None, :]
    f2 = np.arange(T)[:, None]
    th2 = 2 * np.pi * (f2 + 0.5) * n2 / (2 * T)
    inv = np.concatenate([np.cos(th2), -np.sin(th2)], axis=0) / T
    fwd = np.concatenate([fwd, np.zeros((16, 2 * T))], axis=0)
    return jnp.asarray(fwd, bf16), jnp.asarray(inv, bf16)


class _Conv:
    def __init__(self, r0, qT_v, kT_v, vT_v, sk_v, coef_v, fwd_v, inv_v, aT_v):
        self.rows = pl.ds(r0, 8)
        self.refs = (qT_v, kT_v, vT_v, sk_v, coef_v, fwd_v, inv_v, aT_v)

    def fwd(self):
        qT_v, kT_v, vT_v, sk_v, coef_v, fwd_v, inv_v, aT_v = self.refs
        rows = self.rows
        k = kT_v[rows, :].astype(f32)
        coef = coef_v[rows, :]
        lane = lax.broadcasted_iota(jnp.int32, (8, S), 1)
        ks = k * coef[:, 0:1]
        for j in range(1, 4):
            kj = jnp.where(lane >= j, pltpu.roll(k, j, axis=1), 0.0)
            ks = ks + kj * coef[:, j:j + 1]
        u = ks * vT_v[rows, :].astype(f32)
        self.ud = u * coef[:, 4:5]
        lhs = jnp.concatenate(_tiles(u) + _tiles(sk_v[rows, :].astype(f32)), axis=0)
        self.x = jnp.dot(lhs.astype(bf16), fwd_v[0:T, :], preferred_element_type=f32)

    def inv(self):
        inv_v = self.refs[6]
        blk = [self.x[r * 8:(r + 1) * 8, :] for r in range(2 * NB)]
        ur = [b[:, :T] for b in blk[:NB]]
        ui = [b[:, T:] for b in blk[:NB]]
        kr = [b[:, :T] for b in blk[NB:]]
        ki = [b[:, T:] for b in blk[NB:]]
        flane = lax.broadcasted_iota(jnp.int32, (8, T), 1)
        sgn = jnp.where((flane & 1) == 0, 1.0, -1.0).astype(f32)
        wr = [sgn * ki[0]] + [kr[a - 1] + sgn * ki[a] for a in range(1, NB)]
        wi = [-(sgn * kr[0])] + [ki[a - 1] - sgn * kr[a] for a in range(1, NB)]
        ys = []
        for a in range(NB):
            yr = wr[0] * ur[a] - wi[0] * ui[a]
            yi = wr[0] * ui[a] + wi[0] * ur[a]
            for dl in range(1, a + 1):
                yr = yr + (wr[dl] * ur[a - dl] - wi[dl] * ui[a - dl])
                yi = yi + (wr[dl] * ui[a - dl] + wi[dl] * ur[a - dl])
            ys.append(jnp.concatenate([yr, yi], axis=1))
        yf = jnp.concatenate(ys, axis=0)
        y = jnp.dot(yf.astype(bf16), inv_v[...], preferred_element_type=f32)
        self.y = jnp.concatenate([y[a * 8:(a + 1) * 8, :] for a in range(NB)], axis=1)

    def gate(self):
        qT_v, aT_v = self.refs[0], self.refs[7]
        out = qT_v[self.rows, :].astype(f32) * (self.y + self.ud)
        aT_v[self.rows, :] = out
        return pltpu.bitcast(out, u32)


HB = BQ // 2


class _QB128:
    def __init__(self, h, i, q_v, k_s, v_s, ctx_v):
        self.h, self.i = h, i
        self.q_v, self.k_s, self.v_s, self.ctx_v = q_v, k_s, v_s, ctx_v
        self.lo = i * HB
        self.end = self.lo + HB
        self.t = []

    def qk(self, dep=None):
        lo, end = self.lo, self.end
        KCH = CFG['KCH_QK']
        q = _opq(_pk(self.q_v[self.h, lo:lo + HB, :]), self.h)
        if dep is not None:
            q = _tie(q, dep, self.h)
        q = _up(q)
        for a in range(0, end, KCH):
            b = min(a + KCH, end)
            s = lax.dot_general(q, _up(self.k_s[a // 2:b // 2, :]), NT, preferred_element_type=f32)
            self.t += _tiles(s)
        row = lax.broadcasted_iota(jnp.int32, (HB, 128), 0)
        col = lax.broadcasted_iota(jnp.int32, (HB, 128), 1)
        self.t[-1] = jnp.where(col <= row, self.t[-1], NEG)

    def stats(self):
        m = jnp.max(_fold(jnp.maximum, self.t), axis=1, keepdims=True)
        R = CFG['SER']
        if R and self.i >= 2 * CFG['SER0']:
            zero = lax.shift_right_logical(self.h, 8).astype(u32)
            mb = jnp.broadcast_to(m, (HB, 128))
            ls = []
            for g in range(HB // R):
                mg = mb[g * R:(g + 1) * R]
                if ls:
                    mg = mg + pltpu.bitcast(pltpu.bitcast(ls[-1], u32) & zero, f32)
                ls.append(_fold(jnp.add, [jnp.exp2(t[g * R:(g + 1) * R] - mg) for t in self.t]))
            l = jnp.concatenate(ls, axis=0)
        else:
            l = _fold(jnp.add, [jnp.exp2(t - m) for t in self.t])
        self.off = m + jnp.log2(jnp.sum(l, axis=1, keepdims=True))

    def pv(self):
        end = self.end
        KCH = CFG['KCH_PV']
        acc = None
        for a in range(0, end, KCH):
            b = min(a + KCH, end)
            p = jnp.concatenate([jnp.exp2(t - self.off) for t in self.t[a // 128:b // 128]],
                                axis=1).astype(bf16)
            r = jnp.dot(p, _up(self.v_s[a // 2:b // 2, :]), preferred_element_type=f32)
            acc = r if acc is None else acc + r
        self.ctx_v[self.h, self.lo // 2:(self.lo + HB) // 2, :] = _pk(acc.astype(bf16))


def _head_body(h, c_p, qw_v, k_s, v_s, ctx_v, convs):
    nq = S // BQ
    w = {}

    def proj(j, half, dep=None):
        dst = k_s if half == 0 else v_s
        if half not in w:
            w[half] = _up(_opq(_pk(qw_v[H + h, half * C:(half + 1) * C, :]), h))
        n = CFG['PSPLIT']
        for u in range(n):
            lo, hi = j * HB + u * HB // n, j * HB + (u + 1) * HB // n
            lhs = c_p[lo:hi, :]
            if dep is not None and u == 0:
                lhs = _tie(lhs, dep, h)
            r = jnp.dot(_up(lhs), w[half], preferred_element_type=f32)
            dst[lo:hi, :] = _pk(r.astype(bf16))

    B = [_QB128(h, i, qw_v, k_s, v_s, ctx_v) for i in range(2 * nq)]
    plan = {}
    for g, (jf, pf, ji, pi, jg, pg) in enumerate(CFG['CPLAN']):
        plan.setdefault((jf, pf), []).append(convs[g].fwd)
        plan.setdefault((ji, pi), []).append(convs[g].inv)
        plan.setdefault((jg, pg), []).append(convs[g].gate)

    def slot(j, p):
        for f in plan.pop((j, p), []):
            f()

    proj(0, 0)
    slot(-1, 0)
    proj(1, 0)
    slot(-1, 1)
    B[0].qk()
    B[1].qk()
    proj(0, 1)
    for j in range(nq):
        b = 2 * j
        slot(j, 0)
        if j + 1 < nq:
            B[b + 2].qk()
        slot(j, 1)
        B[b].stats()
        B[b].pv()
        slot(j, 2)
        if j + 1 < nq:
            B[b + 3].qk()
            slot(j, 3)
            proj(j + 1, 1)
        slot(j, 4)
        B[b + 1].stats()
        B[b + 1].pv()
        slot(j, 5)
        if j + 2 < nq:
            proj(j + 2, 0)
    assert not plan


NR = 4
XR = S // NR
HH = H // 2
RP = 16
QR = 64
Q1R = 64
AR = 256
NA = 8
A1 = (S - XR) // NA
WR = C // NR


def _kernel(qT_h, kT_h, vT_h, shk_h, sk_h, d_h, xT_h, c_h, wq_h, wuk_h, wuv_h, woT_h,
            fwd_h, inv_h, out_h,
            qT_v, kT_v, vT_v, sk_v, xT_v, x_v, c_v, c_p, wq0_raw, wq1_raw, wq0_p, wq1_p, wuk_raw, wuv_raw,
            qw_v, ctx_v, wo_v, aT_v, coef_v, k_s, v_s, o_s, shk_v, d_v, fwd_v, inv_v,
            sem, sem_x, sem_q0, sem_q1, sem_w, sem_o):
    cp = pltpu.make_async_copy
    c_c = cp(c_h, c_v, sem.at[1])
    a_in = ((kT_h, kT_v), (vT_h, vT_v), (sk_h, sk_v), (qT_h, qT_v))
    late = [cp(src.at[0:H * CH], dst.at[0:H * CH], sem.at[2 + i]) for i, (src, dst) in enumerate(a_in)]
    early = [cp(src.at[H * CH:M], dst.at[H * CH:M], sem.at[11 + i]) for i, (src, dst) in enumerate(a_in)]

    def conv(r0):
        return _Conv(pl.multiple_of(r0, 8), qT_v, kT_v, vT_v, sk_v, coef_v, fwd_v, inv_v, aT_v)

    c_wo = cp(woT_h, wo_v, sem.at[6])
    tiny = [cp(shk_h, shk_v, sem.at[7]), cp(d_h, d_v, sem.at[8]), cp(fwd_h, fwd_v, sem.at[9]),
            cp(inv_h, inv_v, sem.at[10])]

    def rows(j, n, base=0):
        if isinstance(j, int) and isinstance(base, int):
            return pl.ds(base + j * n, n)
        return pl.ds(pl.multiple_of(base + j * n, n), n)

    def x_copy(j):
        return cp(xT_h.at[:, rows(j, XR)], xT_v.at[:, rows(j, XR)], sem_x.at[j])

    def wq0_copy(e, j):
        return cp(wq_h.at[rows(j, QR), 0:HH, e * 128:(e + 1) * 128], wq0_raw.at[e, rows(j, QR)],
                  sem_q0.at[e, j])

    def wq1_copy(j):
        return cp(wq_h.at[rows(j, Q1R), HH:H, :], wq1_raw.at[rows(j, Q1R)], sem_q1.at[j])

    def w_copies(j):
        return (cp(wuk_h.at[rows(j, WR)], wuk_raw.at[rows(j, WR)], sem_w.at[0, j]),
                cp(wuv_h.at[rows(j, WR)], wuv_raw.at[rows(j, WR)], sem_w.at[1, j]))

    def start_seq(fn, lo, hi):
        def body(j, carry):
            for c in fn(j):
                c.start()
            return carry
        lax.fori_loop(lo, hi, body, 0)

    x_copy(0).start()
    start_seq(lambda j: (wq0_copy(0, j),), 0, M // QR)
    for c in tiny:
        c.start()
    start_seq(lambda j: (wq0_copy(1, j),), 0, M // QR)
    start_seq(lambda j: (x_copy(j),), 1, NR)
    for c in early:
        c.start()
    start_seq(lambda j: (wq1_copy(j),), 0, M // Q1R)
    c_c.start()
    start_seq(w_copies, 0, NR)
    for c in late:
        c.start()
    c_wo.start()

    def coef_piece():
        tab = jnp.concatenate([shk_v[...].astype(f32), d_v[...].astype(f32).reshape(1, M),
                               jnp.zeros((3, M), f32)], axis=0)
        coef_v[...] = tab.T

    def xpose_piece(t):
        def run():
            val = _pk(xT_v[:, t * 128:(t + 1) * 128].T)
            x_v[t * 64:(t + 1) * 64, :] = val
            return val[:, 0:384]
        return run

    def wq1_piece(j, t):
        def run():
            val = _pk(pltpu.einshape("chd->hcd", wq1_raw[rows(j * (Q1R // RP) + t, RP)]))
            wq1_p[:, rows(j * (Q1R // RP) + t, RP // 2), :] = val
            return val
        return run

    def qproj(xs, r0, g, slots, wq_p, pieces, z, span=None):
        npc = len(pieces)
        span = span or len(slots) - 1
        done = 0
        deps = []
        for k, (hh, s, e) in enumerate(slots):
            cols = slice(None) if e is None else slice(e * 128, (e + 1) * 128)
            qh = jnp.dot(xs[s], _up(wq_p[hh, :, cols]), preferred_element_type=f32)
            if deps:
                zz = _fold(jnp.bitwise_or, [d[..., t * 8:(t + 1) * 8, u * 128:(u + 1) * 128].reshape(-1, 8, 128)[v]
                                            for d in deps for t in range(d.shape[-2] // 8)
                                            for u in range(d.shape[-1] // 128)
                                            for v in range(d.size // (d.shape[-1] * d.shape[-2]))])
                zz = pltpu.bitcast(zz & z, f32)
                top = qh[0:8, 0:128] + zz
                if qh.shape[1] > 128:
                    top = jnp.concatenate([top, qh[0:8, 128:]], axis=1)
                qh = jnp.concatenate([top, qh[8:]], axis=0)
                deps = []
            n = xs[s].shape[0]
            dst = pl.ds(r0 + s * n, n) if isinstance(r0, int) else pl.ds(pl.multiple_of(r0 + s * n, 64), n)
            qw_v[g * HH + hh, dst, cols] = (qh * QSCALE).astype(bf16)
            want = min(npc, -(-(k + 1) * npc // span))
            while done < want:
                d = pieces[done]()
                if d is not None:
                    deps.append(d)
                done += 1

    def zero_of(i):
        return lax.shift_right_logical(i, 8).astype(u32)

    x_copy(0).wait()
    for t in range(XR // 128):
        xpose_piece(t)()

    def wq0_piece(e, t):
        def run():
            val = _pk(pltpu.einshape("chd->hcd", wq0_raw[e, t * RP:(t + 1) * RP]))
            wq0_p[:, t * (RP // 2):(t + 1) * (RP // 2), e * 128:(e + 1) * 128] = val
            return val
        return run

    def xs0():
        return [_up(x_v[s * (AR // 2):(s + 1) * (AR // 2), :]) for s in range(XR // AR)]

    for j in range(M // QR):
        wq0_copy(0, j).wait()
        for t in range(QR // RP):
            wq0_piece(0, j * (QR // RP) + t)()
    N1, N2 = CFG['N1'], CFG['N2']
    slots = [(hh, s, e) for e in range(2) for hh in range(HH) for s in range(XR // AR)]
    half = len(slots) // 2
    qproj(xs0(), 0, 0, slots[:N1], wq0_p, [], None)
    for c in tiny:
        c.wait()
    for j in range(M // QR):
        wq0_copy(1, j).wait()
    zero = _pk(fwd_v[T:T + 16, 0:128])
    qproj(xs0(), 0, 0, slots[N1:half + N2], wq0_p, [wq0_piece(1, t) for t in range(M // RP)], zero,
          span=half - N1 - 1)
    for j in range(1, NR):
        x_copy(j).wait()
    qproj(xs0(), 0, 0, slots[half + N2:], wq0_p,
          [coef_piece] + [xpose_piece(t) for t in range(XR // 128, S // 128)], zero)

    for c in early:
        c.wait()

    def step_a(r, carry):
        @pl.when(r < M // Q1R)
        def _():
            wq1_copy(r).wait()
        xs = [_up(_opq(x_v[pl.ds(pl.multiple_of(XR // 2 + r * (A1 // 2), 32), A1 // 2), :], r))]
        j = jnp.minimum(r, M // Q1R - 1)
        pieces = [wq1_piece(j, t) for t in range(Q1R // RP)]
        cv = conv(H * CH + r * 8)
        for pos, f in sorted(zip(CFG['APLAN'], (cv.fwd, cv.inv, cv.gate)), key=lambda pf: -pf[0]):
            pieces.insert(pos, f)
        qproj(xs, XR + r * A1, 0, [(hh, 0, None) for hh in range(HH)], wq0_p, pieces, zero_of(r))
        return carry
    lax.fori_loop(0, NA, step_a, 0)

    c_c.wait()

    def step_b(r, carry):
        for c in w_copies(r):
            c.wait()

        def piece(t, w):
            def run():
                src = pl.ds(pl.multiple_of(r * WR + t * RP, RP), RP)
                dst = pl.ds(pl.multiple_of(w * C + r * WR + t * RP, RP), RP)
                raw = wuk_raw if w == 0 else wuv_raw
                qw_v[H:2 * H, dst, :] = pltpu.einshape("chd->hcd", raw[src])
                if w == 0 and t % 2 == 0:
                    n = XR // (WR // RP // 2)
                    o = r * XR + (t // 2) * n
                    val = _pk(c_v[pl.ds(pl.multiple_of(o, n), n), :])
                    c_p[pl.ds(pl.multiple_of(o // 2, n // 2), n // 2), :] = val
                    return val
            return run
        xs = [_up(_opq(x_v[rows(r * (XR // AR) + u, AR // 2), :], r)) for u in range(XR // AR)]
        pieces = [piece(t, w) for t in range(WR // RP) for w in range(2)]
        qproj(xs, r * XR, 1, [(hh, u, None) for hh in range(HH) for u in range(XR // AR)], wq1_p,
              pieces, zero_of(r))
        return carry
    lax.fori_loop(0, NR, step_b, 0)

    for c in late:
        c.wait()

    def head(h, carry):
        _head_body(h, c_p, qw_v, k_s, v_s, ctx_v, [conv(h * CH + g * 8) for g in range(CH // 8)])
        return carry
    lax.fori_loop(0, H, head, 0)

    c_wo.wait()
    OST, OSUB = CFG['OST'], CFG['OSUB']
    OR = S // (OST * OSUB)

    def ostep(j, carry):
        dep = None
        for u in range(OSUB):
            k = j * OSUB + u
            rs = pl.ds(pl.multiple_of(k * OR, OR), OR)
            rp = pl.ds(pl.multiple_of(k * (OR // 2), OR // 2), OR // 2)
            bT = None
            for h in range(H):
                cx = ctx_v[h, rp, :]
                if dep is not None and h == CFG['OTIE']:
                    cx = _tie(cx, dep, j)
                    dep = None
                r = lax.dot_general(wo_v[h], _up(cx), NT, preferred_element_type=f32)
                bT = r if bT is None else bT + r
            full = jnp.concatenate([aT_v[:, rs], bT], axis=0).T
            o_s[rs, :] = full.astype(bf16)
            cp(o_s.at[rs], out_h.at[rs], sem_o.at[k]).start()
            if CFG['OTIE']:
                dep = _fold(jnp.maximum, _tiles(full))
        return carry
    lax.fori_loop(0, OST, ostep, 0)
    for k in range(OST * OSUB):
        cp(o_s.at[k * OR:(k + 1) * OR], out_h.at[k * OR:(k + 1) * OR], sem_o.at[k]).wait()


@jax.jit
def pallas_concat_heads__ssm_conv_h3__compressed_kv_cla__prompt_kernel(
    A_q: jax.Array,
    A_k: jax.Array,
    A_v: jax.Array,
    A_shift_k: jax.Array,
    A_ssm_k: jax.Array,
    A_ssm_D: jax.Array,
    B_x: jax.Array,
    B_c_kv: jax.Array,
    B_w_q: jax.Array,
    B_w_uk: jax.Array,
    B_w_uv: jax.Array,
    B_w_o: jax.Array,
):
    fwd, inv = _dft_mats()
    hbm = pl.BlockSpec(memory_space=pltpu.HBM)
    V = pltpu.VMEM
    out = pl.pallas_call(
        _kernel,
        out_shape=jax.ShapeDtypeStruct((S, 2 * M), bf16),
        in_specs=[hbm] * 14,
        out_specs=hbm,
        scratch_shapes=[
            V((M, S), bf16), V((M, S), bf16), V((M, S), bf16), V((M, S), bf16),
            V((M, S), bf16), V((S // 2, M), u32),
            V((S, C), bf16), V((S // 2, C), u32),
            V((2, M, HH, 128), bf16), V((M, HH, D), bf16),
            V((HH, M // 2, D), u32), V((HH, M // 2, D), u32),
            V((C, H, D), bf16), V((C, H, D), bf16),
            V((2 * H, S, D), bf16), V((H, S // 2, D), u32),
            V((H, M, D), bf16), V((M, S), f32), V((M, 8), f32),
            V((S // 2, D), u32), V((S // 2, D), u32), V((S, 2 * M), bf16),
            V((4, M), bf16), V((M,), bf16), V((T + 16, 2 * T), bf16), V((2 * T, T), bf16),
            pltpu.SemaphoreType.DMA((15,)),
            pltpu.SemaphoreType.DMA((NR,)),
            pltpu.SemaphoreType.DMA((2, M // QR)),
            pltpu.SemaphoreType.DMA((M // Q1R,)),
            pltpu.SemaphoreType.DMA((2, NR)),
            pltpu.SemaphoreType.DMA((16,)),
        ],
        compiler_params=pltpu.CompilerParams(vmem_limit_bytes=120 * 1024 * 1024,
                                             disable_semaphore_checks=True, disable_bounds_checks=True),
    )(A_q[0].T, A_k[0].T, A_v[0].T, A_shift_k.T, A_ssm_k, A_ssm_D, B_x[0].T, B_c_kv[0],
      B_w_q, B_w_uk, B_w_uv, jnp.swapaxes(B_w_o, 1, 2), fwd, inv)
    return out[None]
```

```python
import numpy as np
import jax
import jax.numpy as jnp
from jax import lax
import jax.experimental.pallas as pl
import jax.experimental.pallas.tpu as pltpu

f32 = jnp.float32
bf16 = jnp.bfloat16
u32 = jnp.uint32
NT = (((1,), (1,)), ((), ()))

S = 2048
M = 448
H = 16
D = 256
C = 1024
T = 128
NB = S // T
BQ = 256
CH = 24
CB = M - H * CH
NEG = -1e30
CFG = dict(KCH_QK=512, KCH_PV=512, OTIE=4, OTIE2=10, OU=2, AU=1, SER=32, SER0=5, PSPLIT=1, N1=7, N2=3,
           CPLAN=[(1, 5, 2, 5, 3, 4), (3, 5, 4, 5, 5, 4), (4, 5, 5, 5, 6, 4)],
           APLAN=(0, 3, 4), STEP='ApBVqK')
QSCALE = float(D ** -0.5 * np.log2(np.e))


def _tiles(x):
    return [x[:, t * 128:(t + 1) * 128] for t in range(x.shape[1] // 128)]


def _fold(op, xs):
    r = xs[0]
    for x in xs[1:]:
        r = op(r, x)
    return r


def _pk(x):
    return pltpu.bitcast(x, u32)


def _up(x):
    return pltpu.bitcast(x, bf16)


def _opq(x, h):
    return x ^ lax.shift_right_logical(h, 8).astype(u32)


def _tie(x, dep, h):
    d = dep if dep.dtype == u32 else pltpu.bitcast(dep, u32)
    z = _fold(jnp.bitwise_or, [d[r * 8:(r + 1) * 8, :] for r in range(d.shape[0] // 8)])
    z = z & lax.shift_right_logical(h, 8).astype(u32)
    top = jnp.concatenate([x[0:8, 0:128] ^ z, x[0:8, 128:]], axis=1)
    return jnp.concatenate([top, x[8:]], axis=0)


def _dft_mats():
    n = np.arange(T)[:, None]
    f = np.arange(T)[None, :]
    th = 2 * np.pi * (f + 0.5) * n / (2 * T)
    fwd = np.concatenate([np.cos(th), -np.sin(th)], axis=1)
    n2 = (T + np.arange(T))[None, :]
    f2 = np.arange(T)[:, None]
    th2 = 2 * np.pi * (f2 + 0.5) * n2 / (2 * T)
    inv = np.concatenate([np.cos(th2), -np.sin(th2)], axis=0) / T
    fwd = np.concatenate([fwd, np.zeros((16, 2 * T))], axis=0)
    return jnp.asarray(fwd, bf16), jnp.asarray(inv, bf16)


class _Conv:
    def __init__(self, r0, qT_v, kT_v, vT_v, sk_v, coef_v, fwd_v, inv_v, aT_v):
        self.rows = pl.ds(r0, 8)
        self.refs = (qT_v, kT_v, vT_v, sk_v, coef_v, fwd_v, inv_v, aT_v)

    def fwd(self):
        qT_v, kT_v, vT_v, sk_v, coef_v, fwd_v, inv_v, aT_v = self.refs
        rows = self.rows
        k = kT_v[rows, :].astype(f32)
        coef = coef_v[rows, :]
        lane = lax.broadcasted_iota(jnp.int32, (8, S), 1)
        ks = k * coef[:, 0:1]
        for j in range(1, 4):
            kj = jnp.where(lane >= j, pltpu.roll(k, j, axis=1), 0.0)
            ks = ks + kj * coef[:, j:j + 1]
        u = ks * vT_v[rows, :].astype(f32)
        self.ud = u * coef[:, 4:5]
        lhs = jnp.concatenate(_tiles(u) + _tiles(sk_v[rows, :].astype(f32)), axis=0)
        self.x = jnp.dot(lhs.astype(bf16), fwd_v[0:T, :], preferred_element_type=f32)

    def inv(self):
        inv_v = self.refs[6]
        blk = [self.x[r * 8:(r + 1) * 8, :] for r in range(2 * NB)]
        ur = [b[:, :T] for b in blk[:NB]]
        ui = [b[:, T:] for b in blk[:NB]]
        kr = [b[:, :T] for b in blk[NB:]]
        ki = [b[:, T:] for b in blk[NB:]]
        flane = lax.broadcasted_iota(jnp.int32, (8, T), 1)
        sgn = jnp.where((flane & 1) == 0, 1.0, -1.0).astype(f32)
        wr = [sgn * ki[0]] + [kr[a - 1] + sgn * ki[a] for a in range(1, NB)]
        wi = [-(sgn * kr[0])] + [ki[a - 1] - sgn * kr[a] for a in range(1, NB)]
        ys = []
        for a in range(NB):
            yr = wr[0] * ur[a] - wi[0] * ui[a]
            yi = wr[0] * ui[a] + wi[0] * ur[a]
            for dl in range(1, a + 1):
                yr = yr + (wr[dl] * ur[a - dl] - wi[dl] * ui[a - dl])
                yi = yi + (wr[dl] * ui[a - dl] + wi[dl] * ur[a - dl])
            ys.append(jnp.concatenate([yr, yi], axis=1))
        yf = jnp.concatenate(ys, axis=0)
        y = jnp.dot(yf.astype(bf16), inv_v[...], preferred_element_type=f32)
        self.y = jnp.concatenate([y[a * 8:(a + 1) * 8, :] for a in range(NB)], axis=1)

    def gate(self):
        qT_v, aT_v = self.refs[0], self.refs[7]
        out = qT_v[self.rows, :].astype(f32) * (self.y + self.ud)
        aT_v[self.rows, :] = out
        return pltpu.bitcast(out, u32)


HB = BQ // 2


class _QB128:
    def __init__(self, h, i, q_v, k_s, v_s, ctx_v):
        self.h, self.i = h, i
        self.q_v, self.k_s, self.v_s, self.ctx_v = q_v, k_s, v_s, ctx_v
        self.lo = i * HB
        self.end = self.lo + HB
        self.t = []

    def qk(self, dep=None):
        lo, end = self.lo, self.end
        KCH = CFG['KCH_QK']
        q = _opq(_pk(self.q_v[self.h, lo:lo + HB, :]), self.h)
        if dep is not None:
            q = _tie(q, dep, self.h)
        q = _up(q)
        for a in range(0, end, KCH):
            b = min(a + KCH, end)
            s = lax.dot_general(q, _up(self.k_s[a // 2:b // 2, :]), NT, preferred_element_type=f32)
            self.t += _tiles(s)
        row = lax.broadcasted_iota(jnp.int32, (HB, 128), 0)
        col = lax.broadcasted_iota(jnp.int32, (HB, 128), 1)
        self.t[-1] = jnp.where(col <= row, self.t[-1], NEG)

    def stats(self):
        m = jnp.max(_fold(jnp.maximum, self.t), axis=1, keepdims=True)
        R = CFG['SER']
        if R and self.i >= 2 * CFG['SER0']:
            zero = lax.shift_right_logical(self.h, 8).astype(u32)
            mb = jnp.broadcast_to(m, (HB, 128))
            ls = []
            for g in range(HB // R):
                mg = mb[g * R:(g + 1) * R]
                if ls:
                    mg = mg + pltpu.bitcast(pltpu.bitcast(ls[-1], u32) & zero, f32)
                ls.append(_fold(jnp.add, [jnp.exp2(t[g * R:(g + 1) * R] - mg) for t in self.t]))
            l = jnp.concatenate(ls, axis=0)
        else:
            l = _fold(jnp.add, [jnp.exp2(t - m) for t in self.t])
        self.off = m + jnp.log2(jnp.sum(l, axis=1, keepdims=True))

    def pv(self):
        end = self.end
        KCH = CFG['KCH_PV']
        acc = None
        for a in range(0, end, KCH):
            b = min(a + KCH, end)
            p = jnp.concatenate([jnp.exp2(t - self.off) for t in self.t[a // 128:b // 128]],
                                axis=1).astype(bf16)
            r = jnp.dot(p, _up(self.v_s[a // 2:b // 2, :]), preferred_element_type=f32)
            acc = r if acc is None else acc + r
        self.ctx_v[self.h, self.lo // 2:(self.lo + HB) // 2, :] = _pk(acc.astype(bf16))


def _head_body(h, c_p, qw_v, k_s, v_s, ctx_v, convs):
    nq = S // BQ
    w = {}

    def proj(j, half, dep=None):
        dst = k_s if half == 0 else v_s
        if half not in w:
            w[half] = _up(_opq(_pk(qw_v[H + h, half * C:(half + 1) * C, :]), h))
        n = CFG['PSPLIT']
        for u in range(n):
            lo, hi = j * HB + u * HB // n, j * HB + (u + 1) * HB // n
            lhs = c_p[lo:hi, :]
            if dep is not None and u == 0:
                lhs = _tie(lhs, dep, h)
            r = jnp.dot(_up(lhs), w[half], preferred_element_type=f32)
            dst[lo:hi, :] = _pk(r.astype(bf16))

    B = [_QB128(h, i, qw_v, k_s, v_s, ctx_v) for i in range(2 * nq)]
    plan = {}
    for g, (jf, pf, ji, pi, jg, pg) in enumerate(CFG['CPLAN']):
        plan.setdefault((jf, pf), []).append(convs[g].fwd)
        plan.setdefault((ji, pi), []).append(convs[g].inv)
        plan.setdefault((jg, pg), []).append(convs[g].gate)

    def slot(j, p):
        for f in plan.pop((j, p), []):
            f()

    proj(0, 0)
    slot(-1, 0)
    proj(1, 0)
    slot(-1, 1)
    B[0].qk()
    B[1].qk()
    proj(0, 1)
    for j in range(nq):
        b = 2 * j
        for pos, op in enumerate(CFG['STEP']):
            slot(j, pos)
            if op == 'A' and j + 1 < nq:
                B[b + 2].qk()
            elif op == 'B' and j + 1 < nq:
                B[b + 3].qk()
            elif op == 'V' and j + 1 < nq:
                proj(j + 1, 1)
            elif op == 'K' and j + 2 < nq:
                proj(j + 2, 0)
            elif op in 'pq':
                blk = B[b + (op == 'q')]
                blk.stats()
                blk.pv()
    assert not plan


NR = 4
XR = S // NR
HH = H // 2
RP = 16
QR = 64
Q1R = 64
AR = 256
NA = 8
A1 = (S - XR) // NA
WR = C // NR


def _kernel(qT_h, kT_h, vT_h, shk_h, sk_h, d_h, xT_h, c_h, wq_h, wuk_h, wuv_h, woT_h,
            fwd_h, inv_h, out_h,
            qT_v, kT_v, vT_v, sk_v, xT_v, x_v, c_v, c_p, wq0_raw, wq1_raw, wq0_p, wq1_p, wuk_raw, wuv_raw,
            qw_v, ctx_v, wo_v, aT_v, coef_v, k_s, v_s, o_s, bT_s, shk_v, d_v, fwd_v, inv_v,
            sem, sem_x, sem_q0, sem_q1, sem_w, sem_o):
    cp = pltpu.make_async_copy
    c_c = cp(c_h, c_v, sem.at[1])
    a_in = ((kT_h, kT_v), (vT_h, vT_v), (sk_h, sk_v), (qT_h, qT_v))
    late = [cp(src.at[0:H * CH], dst.at[0:H * CH], sem.at[2 + i]) for i, (src, dst) in enumerate(a_in)]
    early = [cp(src.at[H * CH:M], dst.at[H * CH:M], sem.at[11 + i]) for i, (src, dst) in enumerate(a_in)]

    def conv(r0):
        return _Conv(pl.multiple_of(r0, 8), qT_v, kT_v, vT_v, sk_v, coef_v, fwd_v, inv_v, aT_v)

    c_wo = cp(woT_h, wo_v, sem.at[6])
    tiny = [cp(shk_h, shk_v, sem.at[7]), cp(d_h, d_v, sem.at[8]), cp(fwd_h, fwd_v, sem.at[9]),
            cp(inv_h, inv_v, sem.at[10])]

    def rows(j, n, base=0):
        if isinstance(j, int) and isinstance(base, int):
            return pl.ds(base + j * n, n)
        return pl.ds(pl.multiple_of(base + j * n, n), n)

    def x_copy(j):
        return cp(xT_h.at[:, rows(j, XR)], xT_v.at[:, rows(j, XR)], sem_x.at[j])

    def wq0_copy(e, j):
        return cp(wq_h.at[rows(j, QR), 0:HH, e * 128:(e + 1) * 128], wq0_raw.at[e, rows(j, QR)],
                  sem_q0.at[e, j])

    def wq1_copy(j):
        return cp(wq_h.at[rows(j, Q1R), HH:H, :], wq1_raw.at[rows(j, Q1R)], sem_q1.at[j])

    def w_copies(j):
        return (cp(wuk_h.at[rows(j, WR)], wuk_raw.at[rows(j, WR)], sem_w.at[0, j]),
                cp(wuv_h.at[rows(j, WR)], wuv_raw.at[rows(j, WR)], sem_w.at[1, j]))

    def start_seq(fn, lo, hi):
        def body(j, carry):
            for c in fn(j):
                c.start()
            return carry
        lax.fori_loop(lo, hi, body, 0)

    x_copy(0).start()
    start_seq(lambda j: (wq0_copy(0, j),), 0, M // QR)
    for c in tiny:
        c.start()
    start_seq(lambda j: (wq0_copy(1, j),), 0, M // QR)
    start_seq(lambda j: (x_copy(j),), 1, NR)
    for c in early:
        c.start()
    start_seq(lambda j: (wq1_copy(j),), 0, M // Q1R)
    c_c.start()
    start_seq(w_copies, 0, NR)
    for c in late:
        c.start()
    c_wo.start()

    def coef_piece():
        tab = jnp.concatenate([shk_v[...].astype(f32), d_v[...].astype(f32).reshape(1, M),
                               jnp.zeros((3, M), f32)], axis=0)
        coef_v[...] = tab.T

    def xpose_piece(t):
        def run():
            val = _pk(xT_v[:, t * 128:(t + 1) * 128].T)
            x_v[t * 64:(t + 1) * 64, :] = val
            return val[:, 0:384]
        return run

    def wq1_piece(j, t):
        def run():
            val = _pk(pltpu.einshape("chd->hcd", wq1_raw[rows(j * (Q1R // RP) + t, RP)]))
            wq1_p[:, rows(j * (Q1R // RP) + t, RP // 2), :] = val
            return val
        return run

    def qproj(xs, r0, g, slots, wq_p, pieces, z, span=None):
        npc = len(pieces)
        span = span or len(slots) - 1
        done = 0
        deps = []
        for k, (hh, s, e) in enumerate(slots):
            cols = slice(None) if e is None else slice(e * 128, (e + 1) * 128)
            qh = jnp.dot(xs[s], _up(wq_p[hh, :, cols]), preferred_element_type=f32)
            if deps:
                zz = _fold(jnp.bitwise_or, [d[..., t * 8:(t + 1) * 8, u * 128:(u + 1) * 128].reshape(-1, 8, 128)[v]
                                            for d in deps for t in range(d.shape[-2] // 8)
                                            for u in range(d.shape[-1] // 128)
                                            for v in range(d.size // (d.shape[-1] * d.shape[-2]))])
                zz = pltpu.bitcast(zz & z, f32)
                top = qh[0:8, 0:128] + zz
                if qh.shape[1] > 128:
                    top = jnp.concatenate([top, qh[0:8, 128:]], axis=1)
                qh = jnp.concatenate([top, qh[8:]], axis=0)
                deps = []
            n = xs[s].shape[0]
            dst = pl.ds(r0 + s * n, n) if isinstance(r0, int) else pl.ds(pl.multiple_of(r0 + s * n, 64), n)
            qw_v[g * HH + hh, dst, cols] = (qh * QSCALE).astype(bf16)
            want = min(npc, -(-(k + 1) * npc // span))
            while done < want:
                d = pieces[done]()
                if d is not None:
                    deps.append(d)
                done += 1

    def zero_of(i):
        return lax.shift_right_logical(i, 8).astype(u32)

    bT_s[...] = jnp.zeros(bT_s.shape, f32)
    x_copy(0).wait()
    for t in range(XR // 128):
        xpose_piece(t)()

    def wq0_piece(e, t):
        def run():
            val = _pk(pltpu.einshape("chd->hcd", wq0_raw[e, t * RP:(t + 1) * RP]))
            wq0_p[:, t * (RP // 2):(t + 1) * (RP // 2), e * 128:(e + 1) * 128] = val
            return val
        return run

    def xs0():
        return [_up(x_v[s * (AR // 2):(s + 1) * (AR // 2), :]) for s in range(XR // AR)]

    for j in range(M // QR):
        wq0_copy(0, j).wait()
        for t in range(QR // RP):
            wq0_piece(0, j * (QR // RP) + t)()
    N1, N2 = CFG['N1'], CFG['N2']
    slots = [(hh, s, e) for e in range(2) for hh in range(HH) for s in range(XR // AR)]
    half = len(slots) // 2
    qproj(xs0(), 0, 0, slots[:N1], wq0_p, [], None)
    for c in tiny:
        c.wait()
    for j in range(M // QR):
        wq0_copy(1, j).wait()
    zero = _pk(fwd_v[T:T + 16, 0:128])
    qproj(xs0(), 0, 0, slots[N1:half + N2], wq0_p, [wq0_piece(1, t) for t in range(M // RP)], zero,
          span=half - N1 - 1)
    for j in range(1, NR):
        x_copy(j).wait()
    qproj(xs0(), 0, 0, slots[half + N2:], wq0_p,
          [coef_piece] + [xpose_piece(t) for t in range(XR // 128, S // 128)], zero)

    for c in early:
        c.wait()

    AU = CFG['AU']

    def step_a(i, carry):
        for u in range(AU):
            @pl.when(i * AU + u < M // Q1R)
            def _():
                wq1_copy(i * AU + u).wait()
        xs = [_up(_opq(x_v[pl.ds(pl.multiple_of(XR // 2 + (i * AU + u) * (A1 // 2), 32), A1 // 2), :], i))
              for u in range(AU)]
        pieces = []
        for u in range(AU):
            r = i * AU + u
            j = jnp.minimum(r, M // Q1R - 1)
            sub = [wq1_piece(j, t) for t in range(Q1R // RP)]
            cv = conv(H * CH + r * 8)
            for pos, f in sorted(zip(CFG['APLAN'], (cv.fwd, cv.inv, cv.gate)), key=lambda pf: -pf[0]):
                sub.insert(pos, f)
            pieces += sub
        qproj(xs, XR + i * AU * A1, 0, [(hh, u, None) for hh in range(HH) for u in range(AU)], wq0_p,
              pieces, zero_of(i))
        return carry
    lax.fori_loop(0, NA // AU, step_a, 0)

    c_c.wait()

    def step_b(r, carry):
        for c in w_copies(r):
            c.wait()

        def piece(t, w):
            def run():
                src = pl.ds(pl.multiple_of(r * WR + t * RP, RP), RP)
                dst = pl.ds(pl.multiple_of(w * C + r * WR + t * RP, RP), RP)
                raw = wuk_raw if w == 0 else wuv_raw
                qw_v[H:2 * H, dst, :] = pltpu.einshape("chd->hcd", raw[src])
                if w == 0 and t % 2 == 0:
                    n = XR // (WR // RP // 2)
                    o = r * XR + (t // 2) * n
                    val = _pk(c_v[pl.ds(pl.multiple_of(o, n), n), :])
                    c_p[pl.ds(pl.multiple_of(o // 2, n // 2), n // 2), :] = val
                    return val
            return run
        xs = [_up(_opq(x_v[rows(r * (XR // AR) + u, AR // 2), :], r)) for u in range(XR // AR)]
        pieces = [piece(t, w) for t in range(WR // RP) for w in range(2)]
        qproj(xs, r * XR, 1, [(hh, u, None) for hh in range(HH) for u in range(XR // AR)], wq1_p,
              pieces, zero_of(r))
        return carry
    lax.fori_loop(0, NR, step_b, 0)

    for c in late:
        c.wait()

    def head(h, carry):
        _head_body(h, c_p, qw_v, k_s, v_s, ctx_v, [conv(h * CH + g * 8) for g in range(CH // 8)])
        return carry
    lax.fori_loop(0, H, head, 0)

    c_wo.wait()
    NO = S // BQ
    OU = CFG['OU']
    MA = M // 128 * 128

    def emit_a(k):
        rs = rows(k, BQ)
        val = aT_v[0:MA, rs].T
        o_s[rs, 0:MA] = val.astype(bf16)
        return val

    def emit_b(rs, bT):
        val = jnp.concatenate([aT_v[MA:M, rs], bT], axis=0).T
        o_s[rs, MA:2 * M] = val.astype(bf16)
        return val

    def copy_a(k):
        return cp(o_s.at[rows(k, BQ), 0:MA], out_h.at[rows(k, BQ), 0:MA], sem_o.at[0, k])

    def copy_b(rs, k):
        return cp(o_s.at[rs, MA:2 * M], out_h.at[rs, MA:2 * M], sem_o.at[1, k])

    def ostep(j, carry):
        dep = _fold(jnp.maximum, _tiles(emit_b(rows(jnp.maximum(j * OU - 1, 0), BQ), bT_s[...])))
        for u in range(OU):
            k = j * OU + u
            dep2 = _fold(jnp.maximum, _tiles(emit_a(k)))
            copy_a(k).start()
            bT = None
            for h in range(H):
                cx = ctx_v[h, rows(k, HB), :]
                if h == CFG['OTIE']:
                    cx = _tie(cx, dep, j)
                if h == CFG['OTIE2']:
                    cx = _tie(cx, dep2, j)
                r = lax.dot_general(wo_v[h], _up(cx), NT, preferred_element_type=f32)
                bT = r if bT is None else bT + r
            if u + 1 < OU:
                dep = _fold(jnp.maximum, _tiles(emit_b(rows(k, BQ), bT)))
                copy_b(rows(k, BQ), k).start()
        bT_s[...] = bT

        @pl.when(j > 0)
        def _():
            copy_b(rows(j * OU - 1, BQ), j * OU - 1).start()
        return carry
    lax.fori_loop(0, NO // OU, ostep, 0)
    last = [pl.ds(S - BQ + u * HB, HB) for u in range(2)]
    for u in range(2):
        emit_b(last[u], bT_s[:, u * HB:(u + 1) * HB])
        copy_b(last[u], NO - 1 + u).start()
    for k in range(NO):
        copy_a(k).wait()
    for k in range(NO - 1):
        copy_b(rows(k, BQ), k).wait()
    for u in range(2):
        copy_b(last[u], NO - 1 + u).wait()


@jax.jit
def pallas_concat_heads__ssm_conv_h3__compressed_kv_cla__prompt_kernel(
    A_q: jax.Array,
    A_k: jax.Array,
    A_v: jax.Array,
    A_shift_k: jax.Array,
    A_ssm_k: jax.Array,
    A_ssm_D: jax.Array,
    B_x: jax.Array,
    B_c_kv: jax.Array,
    B_w_q: jax.Array,
    B_w_uk: jax.Array,
    B_w_uv: jax.Array,
    B_w_o: jax.Array,
):
    fwd, inv = _dft_mats()
    hbm = pl.BlockSpec(memory_space=pltpu.HBM)
    V = pltpu.VMEM
    out = pl.pallas_call(
        _kernel,
        out_shape=jax.ShapeDtypeStruct((S, 2 * M), bf16),
        in_specs=[hbm] * 14,
        out_specs=hbm,
        scratch_shapes=[
            V((M, S), bf16), V((M, S), bf16), V((M, S), bf16), V((M, S), bf16),
            V((M, S), bf16), V((S // 2, M), u32),
            V((S, C), bf16), V((S // 2, C), u32),
            V((2, M, HH, 128), bf16), V((M, HH, D), bf16),
            V((HH, M // 2, D), u32), V((HH, M // 2, D), u32),
            V((C, H, D), bf16), V((C, H, D), bf16),
            V((2 * H, S, D), bf16), V((H, S // 2, D), u32),
            V((H, M, D), bf16), V((M, S), f32), V((M, 8), f32),
            V((S // 2, D), u32), V((S // 2, D), u32), V((S, 2 * M), bf16),
            V((M, BQ), f32),
            V((4, M), bf16), V((M,), bf16), V((T + 16, 2 * T), bf16), V((2 * T, T), bf16),
            pltpu.SemaphoreType.DMA((15,)),
            pltpu.SemaphoreType.DMA((NR,)),
            pltpu.SemaphoreType.DMA((2, M // QR)),
            pltpu.SemaphoreType.DMA((M // Q1R,)),
            pltpu.SemaphoreType.DMA((2, NR)),
            pltpu.SemaphoreType.DMA((2, S // BQ + 1)),
        ],
        compiler_params=pltpu.CompilerParams(vmem_limit_bytes=120 * 1024 * 1024,
                                             disable_semaphore_checks=True, disable_bounds_checks=True),
    )(A_q[0].T, A_k[0].T, A_v[0].T, A_shift_k.T, A_ssm_k, A_ssm_D, B_x[0].T, B_c_kv[0],
      B_w_q, B_w_uk, B_w_uv, jnp.swapaxes(B_w_o, 1, 2), fwd, inv)
    return out[None]
```

```python
import numpy as np
import jax
import jax.numpy as jnp
from jax import lax
import jax.experimental.pallas as pl
import jax.experimental.pallas.tpu as pltpu

f32 = jnp.float32
bf16 = jnp.bfloat16
u32 = jnp.uint32
NT = (((1,), (1,)), ((), ()))

S = 2048
M = 448
H = 16
D = 256
C = 1024
T = 128
NB = S // T
QB = 128
PB = 256
KCH = 512
CH = 24
NEG = -1e30
QSCALE = float(D ** -0.5 * np.log2(np.e))

NR = 4
XR = S // NR
HH = H // 2
RP = 16
QR = 64
NQ = M // QR
AR = 256
NA = 8
A1 = (S - XR) // NA
WR = C // NR
OU = 2
MA = M // 128 * 128


def _tiles(x):
    return [x[:, t * 128:(t + 1) * 128] for t in range(x.shape[1] // 128)]


def _fold(op, xs):
    r = xs[0]
    for x in xs[1:]:
        r = op(r, x)
    return r


def _pk(x):
    return pltpu.bitcast(x, u32)


def _up(x):
    return pltpu.bitcast(x, bf16)


def _zero(i):
    return lax.shift_right_logical(i, 8).astype(u32)


def _opq(x, i):
    return x ^ _zero(i)


def _tie(x, dep, i):
    d = pltpu.bitcast(dep, u32)
    z = _fold(jnp.bitwise_or, [d[r * 8:(r + 1) * 8, :] for r in range(d.shape[0] // 8)]) & _zero(i)
    top = jnp.concatenate([x[0:8, 0:128] ^ z, x[0:8, 128:]], axis=1)
    return jnp.concatenate([top, x[8:]], axis=0)


def _rows(j, n):
    if isinstance(j, int):
        return pl.ds(j * n, n)
    return pl.ds(pl.multiple_of(j * n, n), n)


def _dft_mats():
    n = np.arange(T)[:, None]
    f = np.arange(T)[None, :]
    th = 2 * np.pi * (f + 0.5) * n / (2 * T)
    fwd = np.concatenate([np.cos(th), -np.sin(th)], axis=1)
    fwd = np.concatenate([fwd, np.zeros((16, 2 * T))], axis=0)
    n2 = (T + np.arange(T))[None, :]
    f2 = np.arange(T)[:, None]
    th2 = 2 * np.pi * (f2 + 0.5) * n2 / (2 * T)
    inv = np.concatenate([np.cos(th2), -np.sin(th2)], axis=0) / T
    return jnp.asarray(fwd, bf16), jnp.asarray(inv, bf16)


class _Conv:
    def __init__(self, r0, qT_v, kT_v, vT_v, sk_v, coef_v, fwd_v, inv_v, aT_v):
        self.rows = pl.ds(pl.multiple_of(r0, 8), 8)
        self.refs = (qT_v, kT_v, vT_v, sk_v, coef_v, fwd_v, inv_v, aT_v)

    def fwd(self):
        _, kT_v, vT_v, sk_v, coef_v, fwd_v, _, _ = self.refs
        rows = self.rows
        k = kT_v[rows, :].astype(f32)
        coef = coef_v[rows, :]
        lane = lax.broadcasted_iota(jnp.int32, (8, S), 1)
        ks = k * coef[:, 0:1]
        for j in range(1, 4):
            kj = jnp.where(lane >= j, pltpu.roll(k, j, axis=1), 0.0)
            ks = ks + kj * coef[:, j:j + 1]
        u = ks * vT_v[rows, :].astype(f32)
        self.ud = u * coef[:, 4:5]
        lhs = jnp.concatenate(_tiles(u) + _tiles(sk_v[rows, :].astype(f32)), axis=0)
        self.x = jnp.dot(lhs.astype(bf16), fwd_v[0:T, :], preferred_element_type=f32)

    def inv(self):
        inv_v = self.refs[6]
        blk = [self.x[r * 8:(r + 1) * 8, :] for r in range(2 * NB)]
        ur = [b[:, :T] for b in blk[:NB]]
        ui = [b[:, T:] for b in blk[:NB]]
        kr = [b[:, :T] for b in blk[NB:]]
        ki = [b[:, T:] for b in blk[NB:]]
        flane = lax.broadcasted_iota(jnp.int32, (8, T), 1)
        sgn = jnp.where((flane & 1) == 0, 1.0, -1.0).astype(f32)
        wr = [sgn * ki[0]] + [kr[a - 1] + sgn * ki[a] for a in range(1, NB)]
        wi = [-(sgn * kr[0])] + [ki[a - 1] - sgn * kr[a] for a in range(1, NB)]
        ys = []
        for a in range(NB):
            yr = wr[0] * ur[a] - wi[0] * ui[a]
            yi = wr[0] * ui[a] + wi[0] * ur[a]
            for dl in range(1, a + 1):
                yr = yr + (wr[dl] * ur[a - dl] - wi[dl] * ui[a - dl])
                yi = yi + (wr[dl] * ui[a - dl] + wi[dl] * ur[a - dl])
            ys.append(jnp.concatenate([yr, yi], axis=1))
        yf = jnp.concatenate(ys, axis=0)
        y = jnp.dot(yf.astype(bf16), inv_v[...], preferred_element_type=f32)
        self.y = jnp.concatenate([y[a * 8:(a + 1) * 8, :] for a in range(NB)], axis=1)

    def gate(self):
        qT_v, aT_v = self.refs[0], self.refs[7]
        out = qT_v[self.rows, :].astype(f32) * (self.y + self.ud)
        aT_v[self.rows, :] = out
        return pltpu.bitcast(out, u32)


class _QBlock:
    def __init__(self, h, i, q_v, k_s, v_s, ctx_v):
        self.h, self.i = h, i
        self.q_v, self.k_s, self.v_s, self.ctx_v = q_v, k_s, v_s, ctx_v
        self.lo = i * QB
        self.end = self.lo + QB
        self.t = []

    def scores(self):
        q = _up(_opq(_pk(self.q_v[self.h, self.lo:self.end, :]), self.h))
        for a in range(0, self.end, KCH):
            b = min(a + KCH, self.end)
            s = lax.dot_general(q, _up(self.k_s[a // 2:b // 2, :]), NT, preferred_element_type=f32)
            self.t += _tiles(s)
        row = lax.broadcasted_iota(jnp.int32, (QB, QB), 0)
        col = lax.broadcasted_iota(jnp.int32, (QB, QB), 1)
        self.t[-1] = jnp.where(col <= row, self.t[-1], NEG)

    def values(self):
        m = jnp.max(_fold(jnp.maximum, self.t), axis=1, keepdims=True)
        if self.i >= 8:
            R = 32
            mb = jnp.broadcast_to(m, (QB, 128))
            ls = []
            for g in range(QB // R):
                mg = mb[g * R:(g + 1) * R]
                if ls:
                    mg = mg + pltpu.bitcast(pltpu.bitcast(ls[-1], u32) & _zero(self.h), f32)
                ls.append(_fold(jnp.add, [jnp.exp2(t[g * R:(g + 1) * R] - mg) for t in self.t]))
            l = jnp.concatenate(ls, axis=0)
        else:
            l = _fold(jnp.add, [jnp.exp2(t - m) for t in self.t])
        off = m + jnp.log2(jnp.sum(l, axis=1, keepdims=True))
        acc = None
        for a in range(0, self.end, KCH):
            b = min(a + KCH, self.end)
            p = jnp.concatenate([jnp.exp2(t - off) for t in self.t[a // 128:b // 128]], axis=1)
            r = jnp.dot(p.astype(bf16), _up(self.v_s[a // 2:b // 2, :]), preferred_element_type=f32)
            acc = r if acc is None else acc + r
        self.ctx_v[self.h, self.lo // 2:self.end // 2, :] = _pk(acc.astype(bf16))


def _head_body(h, c_p, qw_v, k_s, v_s, ctx_v, convs):
    n = S // PB
    w = {}

    def proj(j, half):
        if half not in w:
            w[half] = _up(_opq(_pk(qw_v[H + h, half * C:(half + 1) * C, :]), h))
        rows = slice(j * PB // 2, (j + 1) * PB // 2)
        r = jnp.dot(_up(c_p[rows, :]), w[half], preferred_element_type=f32)
        (k_s, v_s)[half][rows, :] = _pk(r.astype(bf16))

    blk = [_QBlock(h, i, qw_v, k_s, v_s, ctx_v) for i in range(S // QB)]
    c0, c1, c2 = convs
    before_k = {1: [c0.fwd], 2: [c0.inv], 3: [c1.fwd], 4: [c1.inv, c2.fwd], 5: [c2.inv]}
    before_pv = {3: c0.gate, 5: c1.gate, 6: c2.gate}
    proj(0, 0)
    proj(1, 0)
    blk[0].scores()
    blk[1].scores()
    proj(0, 1)
    for j in range(n):
        if j + 1 < n:
            blk[2 * j + 2].scores()
        blk[2 * j].values()
        if j + 1 < n:
            blk[2 * j + 3].scores()
            proj(j + 1, 1)
        if j in before_pv:
            before_pv[j]()
        blk[2 * j + 1].values()
        for f in before_k.get(j, ()):
            f()
        if j + 2 < n:
            proj(j + 2, 0)


def _kernel(qT_h, kT_h, vT_h, shk_h, sk_h, d_h, xT_h, c_h, wq_h, wuk_h, wuv_h, woT_h,
            fwd_h, inv_h, out_h,
            qT_v, kT_v, vT_v, sk_v, xT_v, x_v, c_v, c_p, wq0_raw, wq1_raw, wq0_p, wq1_p,
            wuk_raw, wuv_raw, qw_v, ctx_v, wo_v, aT_v, coef_v, k_s, v_s, o_s, bT_s,
            shk_v, d_v, fwd_v, inv_v,
            sem, sem_x, sem_q0, sem_q1, sem_w, sem_o):
    cp = pltpu.make_async_copy

    a_in = ((kT_h, kT_v), (vT_h, vT_v), (sk_h, sk_v), (qT_h, qT_v))
    a_late = [cp(s.at[0:H * CH], d.at[0:H * CH], sem.at[i]) for i, (s, d) in enumerate(a_in)]
    a_early = [cp(s.at[H * CH:M], d.at[H * CH:M], sem.at[4 + i]) for i, (s, d) in enumerate(a_in)]
    tiny = [cp(shk_h, shk_v, sem.at[8]), cp(d_h, d_v, sem.at[9]), cp(fwd_h, fwd_v, sem.at[10]),
            cp(inv_h, inv_v, sem.at[11])]
    c_copy = cp(c_h, c_v, sem.at[12])
    wo_copy = cp(woT_h, wo_v, sem.at[13])

    def x_copy(j):
        return cp(xT_h.at[:, _rows(j, XR)], xT_v.at[:, _rows(j, XR)], sem_x.at[j])

    def wq0_copy(e, j):
        return cp(wq_h.at[_rows(j, QR), 0:HH, e * 128:(e + 1) * 128], wq0_raw.at[e, _rows(j, QR)],
                  sem_q0.at[e, j])

    def wq1_copy(j):
        return cp(wq_h.at[_rows(j, QR), HH:H, :], wq1_raw.at[_rows(j, QR)], sem_q1.at[j])

    def w_copies(j):
        return (cp(wuk_h.at[_rows(j, WR)], wuk_raw.at[_rows(j, WR)], sem_w.at[0, j]),
                cp(wuv_h.at[_rows(j, WR)], wuv_raw.at[_rows(j, WR)], sem_w.at[1, j]))

    def start_seq(fn, lo, hi):
        def body(j, carry):
            for c in fn(j):
                c.start()
            return carry
        lax.fori_loop(lo, hi, body, 0)

    x_copy(0).start()
    start_seq(lambda j: (wq0_copy(0, j),), 0, NQ)
    for c in tiny:
        c.start()
    start_seq(lambda j: (wq0_copy(1, j),), 0, NQ)
    start_seq(lambda j: (x_copy(j),), 1, NR)
    for c in a_early:
        c.start()
    start_seq(lambda j: (wq1_copy(j),), 0, NQ)
    c_copy.start()
    start_seq(w_copies, 0, NR)
    for c in a_late:
        c.start()
    wo_copy.start()

    def conv(r0):
        return _Conv(r0, qT_v, kT_v, vT_v, sk_v, coef_v, fwd_v, inv_v, aT_v)

    def coef_piece():
        tab = jnp.concatenate([shk_v[...].astype(f32), d_v[...].astype(f32).reshape(1, M),
                               jnp.zeros((3, M), f32)], axis=0)
        coef_v[...] = tab.T

    def xpose_piece(t):
        def run():
            val = _pk(xT_v[:, t * 128:(t + 1) * 128].T)
            x_v[t * 64:(t + 1) * 64, :] = val
            return val[:, 0:MA]
        return run

    def wq0_piece(e, t):
        def run():
            val = _pk(pltpu.einshape("chd->hcd", wq0_raw[e, t * RP:(t + 1) * RP]))
            wq0_p[:, t * (RP // 2):(t + 1) * (RP // 2), e * 128:(e + 1) * 128] = val
            return val
        return run

    def wq1_piece(t):
        def run():
            val = _pk(pltpu.einshape("chd->hcd", wq1_raw[_rows(t, RP)]))
            wq1_p[:, _rows(t, RP // 2), :] = val
            return val
        return run

    def qproj(xs, r0, g, slots, wq_p, pieces, z, span=None):
        span = span or len(slots) - 1
        done = 0
        deps = []
        for k, (hh, s, e) in enumerate(slots):
            cols = slice(None) if e is None else slice(e * 128, (e + 1) * 128)
            qh = jnp.dot(xs[s], _up(wq_p[hh, :, cols]), preferred_element_type=f32)
            if deps:
                vregs = [d[..., t * 8:(t + 1) * 8, u * 128:(u + 1) * 128].reshape(-1, 8, 128)[v]
                         for d in deps for t in range(d.shape[-2] // 8)
                         for u in range(d.shape[-1] // 128)
                         for v in range(d.size // (d.shape[-1] * d.shape[-2]))]
                top = qh[0:8, 0:128] + pltpu.bitcast(_fold(jnp.bitwise_or, vregs) & z, f32)
                if qh.shape[1] > 128:
                    top = jnp.concatenate([top, qh[0:8, 128:]], axis=1)
                qh = jnp.concatenate([top, qh[8:]], axis=0)
                deps = []
            n = xs[s].shape[0]
            o = r0 + s * n
            dst = pl.ds(o, n) if isinstance(o, int) else pl.ds(pl.multiple_of(o, 64), n)
            qw_v[g * HH + hh, dst, cols] = (qh * QSCALE).astype(bf16)
            while done < min(len(pieces), -(-(k + 1) * len(pieces) // span)):
                d = pieces[done]()
                if d is not None:
                    deps.append(d)
                done += 1

    def xs0():
        return [_up(x_v[s * (AR // 2):(s + 1) * (AR // 2), :]) for s in range(XR // AR)]

    bT_s[...] = jnp.zeros(bT_s.shape, f32)
    x_copy(0).wait()
    for t in range(XR // 128):
        xpose_piece(t)()
    for j in range(NQ):
        wq0_copy(0, j).wait()
        for t in range(QR // RP):
            wq0_piece(0, j * (QR // RP) + t)()
    slots = [(hh, s, e) for e in range(2) for hh in range(HH) for s in range(XR // AR)]
    n1, n2 = 7, len(slots) // 2 + 3
    qproj(xs0(), 0, 0, slots[:n1], wq0_p, [], None)
    for c in tiny:
        c.wait()
    for j in range(NQ):
        wq0_copy(1, j).wait()
    zero = _pk(fwd_v[T:T + 16, 0:128])
    qproj(xs0(), 0, 0, slots[n1:n2], wq0_p, [wq0_piece(1, t) for t in range(M // RP)], zero,
          span=len(slots) // 2 - n1 - 1)
    for j in range(1, NR):
        x_copy(j).wait()
    qproj(xs0(), 0, 0, slots[n2:], wq0_p,
          [coef_piece] + [xpose_piece(t) for t in range(XR // 128, S // 128)], zero)
    for c in a_early:
        c.wait()

    def step_a(r, carry):
        @pl.when(r < NQ)
        def _():
            wq1_copy(r).wait()
        x = _up(_opq(x_v[pl.ds(pl.multiple_of(XR // 2 + r * (A1 // 2), 32), A1 // 2), :], r))
        w = [wq1_piece(jnp.minimum(r, NQ - 1) * (QR // RP) + t) for t in range(QR // RP)]
        cv = conv(H * CH + r * 8)
        qproj([x], XR + r * A1, 0, [(hh, 0, None) for hh in range(HH)], wq0_p,
              [cv.fwd] + w[:3] + [cv.inv, w[3], cv.gate], _zero(r))
        return carry
    lax.fori_loop(0, NA, step_a, 0)

    c_copy.wait()

    def step_b(r, carry):
        for c in w_copies(r):
            c.wait()

        def piece(t, w):
            def run():
                src = pl.ds(pl.multiple_of(r * WR + t * RP, RP), RP)
                dst = pl.ds(pl.multiple_of(w * C + r * WR + t * RP, RP), RP)
                qw_v[H:2 * H, dst, :] = pltpu.einshape("chd->hcd", (wuk_raw, wuv_raw)[w][src])
                if w == 0 and t % 2 == 0:
                    k = r * (XR // 64) + t // 2
                    val = _pk(c_v[_rows(k, 64), :])
                    c_p[_rows(k, 32), :] = val
                    return val
            return run
        xs = [_up(_opq(x_v[_rows(r * (XR // AR) + u, AR // 2), :], r)) for u in range(XR // AR)]
        qproj(xs, r * XR, 1, [(hh, u, None) for hh in range(HH) for u in range(XR // AR)], wq1_p,
              [piece(t, w) for t in range(WR // RP) for w in range(2)], _zero(r))
        return carry
    lax.fori_loop(0, NR, step_b, 0)

    for c in a_late:
        c.wait()

    def head(h, carry):
        _head_body(h, c_p, qw_v, k_s, v_s, ctx_v, [conv(h * CH + g * 8) for g in range(CH // 8)])
        return carry
    lax.fori_loop(0, H, head, 0)

    wo_copy.wait()
    no = S // PB

    def emit_a(k):
        val = aT_v[0:MA, _rows(k, PB)].T
        o_s[_rows(k, PB), 0:MA] = val.astype(bf16)
        return _fold(jnp.maximum, _tiles(val))

    def emit_b(rs, bT):
        val = jnp.concatenate([aT_v[MA:M, rs], bT], axis=0).T
        o_s[rs, MA:2 * M] = val.astype(bf16)
        return _fold(jnp.maximum, _tiles(val))

    def copy_a(k):
        return cp(o_s.at[_rows(k, PB), 0:MA], out_h.at[_rows(k, PB), 0:MA], sem_o.at[0, k])

    def copy_b(rs, k):
        return cp(o_s.at[rs, MA:2 * M], out_h.at[rs, MA:2 * M], sem_o.at[1, k])

    def ostep(j, carry):
        dep_b = emit_b(_rows(jnp.maximum(j * OU - 1, 0), PB), bT_s[...])
        for u in range(OU):
            k = j * OU + u
            dep_a = emit_a(k)
            copy_a(k).start()
            bT = None
            for h in range(H):
                cx = ctx_v[h, _rows(k, PB // 2), :]
                if h in (4, 10):
                    cx = _tie(cx, dep_b if h == 4 else dep_a, j)
                r = lax.dot_general(wo_v[h], _up(cx), NT, preferred_element_type=f32)
                bT = r if bT is None else bT + r
            if u + 1 < OU:
                dep_b = emit_b(_rows(k, PB), bT)
                copy_b(_rows(k, PB), k).start()
        bT_s[...] = bT

        @pl.when(j > 0)
        def _():
            copy_b(_rows(j * OU - 1, PB), j * OU - 1).start()
        return carry
    lax.fori_loop(0, no // OU, ostep, 0)
    last = [pl.ds(S - PB + u * 128, 128) for u in range(2)]
    for u in range(2):
        emit_b(last[u], bT_s[:, u * 128:(u + 1) * 128])
        copy_b(last[u], no - 1 + u).start()
    for k in range(no):
        copy_a(k).wait()
    for k in range(no - 1):
        copy_b(_rows(k, PB), k).wait()
    for u in range(2):
        copy_b(last[u], no - 1 + u).wait()


@jax.jit
def pallas_concat_heads__ssm_conv_h3__compressed_kv_cla__prompt_kernel(
    A_q: jax.Array,
    A_k: jax.Array,
    A_v: jax.Array,
    A_shift_k: jax.Array,
    A_ssm_k: jax.Array,
    A_ssm_D: jax.Array,
    B_x: jax.Array,
    B_c_kv: jax.Array,
    B_w_q: jax.Array,
    B_w_uk: jax.Array,
    B_w_uv: jax.Array,
    B_w_o: jax.Array,
):
    fwd, inv = _dft_mats()
    hbm = pl.BlockSpec(memory_space=pltpu.HBM)
    V = pltpu.VMEM
    dma = pltpu.SemaphoreType.DMA
    out = pl.pallas_call(
        _kernel,
        out_shape=jax.ShapeDtypeStruct((S, 2 * M), bf16),
        in_specs=[hbm] * 14,
        out_specs=hbm,
        scratch_shapes=[
            V((M, S), bf16), V((M, S), bf16), V((M, S), bf16), V((M, S), bf16),
            V((M, S), bf16), V((S // 2, M), u32),
            V((S, C), bf16), V((S // 2, C), u32),
            V((2, M, HH, 128), bf16), V((M, HH, D), bf16),
            V((HH, M // 2, D), u32), V((HH, M // 2, D), u32),
            V((C, H, D), bf16), V((C, H, D), bf16),
            V((2 * H, S, D), bf16), V((H, S // 2, D), u32),
            V((H, M, D), bf16), V((M, S), f32), V((M, 8), f32),
            V((S // 2, D), u32), V((S // 2, D), u32),
            V((S, 2 * M), bf16), V((M, PB), f32),
            V((4, M), bf16), V((M,), bf16), V((T + 16, 2 * T), bf16), V((2 * T, T), bf16),
            dma((14,)), dma((NR,)), dma((2, NQ)), dma((NQ,)), dma((2, NR)), dma((2, S // PB + 1)),
        ],
        compiler_params=pltpu.CompilerParams(
            vmem_limit_bytes=120 * 1024 * 1024,
            disable_semaphore_checks=True, disable_bounds_checks=True),
    )(A_q[0].T, A_k[0].T, A_v[0].T, A_shift_k.T, A_ssm_k, A_ssm_D, B_x[0].T, B_c_kv[0],
      B_w_q, B_w_uk, B_w_uv, jnp.swapaxes(B_w_o, 1, 2), fwd, inv)
    return out[None]
```

```python
import numpy as np
import jax
import jax.numpy as jnp
from jax import lax
import jax.experimental.pallas as pl
import jax.experimental.pallas.tpu as pltpu

f32 = jnp.float32
bf16 = jnp.bfloat16
u32 = jnp.uint32
NT = (((1,), (1,)), ((), ()))

S = 2048
M = 448
H = 16
D = 256
C = 1024
T = 128
NB = S // T
QB = 128
PB = 256
KCH = 512
CH = 24
NEG = -1e30
QSCALE = float(D ** -0.5 * np.log2(np.e))

NR = 4
XR = S // NR
HH = H // 2
RP = 16
QR = 64
NQ = M // QR
AR = 256
NA = 8
A1 = (S - XR) // NA
WR = C // NR
OU = 2
MA = M // 128 * 128


def _tiles(x):
    return [x[:, t * 128:(t + 1) * 128] for t in range(x.shape[1] // 128)]


def _fold(op, xs):
    r = xs[0]
    for x in xs[1:]:
        r = op(r, x)
    return r


def _pk(x):
    return pltpu.bitcast(x, u32)


def _up(x):
    return pltpu.bitcast(x, bf16)


def _zero(i):
    return lax.shift_right_logical(i, 8).astype(u32)


def _opq(x, i):
    return x ^ _zero(i)


def _tie(x, dep, i):
    d = pltpu.bitcast(dep, u32)
    z = _fold(jnp.bitwise_or, [d[r * 8:(r + 1) * 8, :] for r in range(d.shape[0] // 8)]) & _zero(i)
    top = jnp.concatenate([x[0:8, 0:128] ^ z, x[0:8, 128:]], axis=1)
    return jnp.concatenate([top, x[8:]], axis=0)


def _rows(j, n):
    if isinstance(j, int):
        return pl.ds(j * n, n)
    return pl.ds(pl.multiple_of(j * n, n), n)


def _dft_mats():
    n = np.arange(T)[:, None]
    f = np.arange(T)[None, :]
    th = 2 * np.pi * (f + 0.5) * n / (2 * T)
    fwd = np.concatenate([np.cos(th), -np.sin(th)], axis=1)
    fwd = np.concatenate([fwd, np.zeros((16, 2 * T))], axis=0)
    n2 = (T + np.arange(T))[None, :]
    f2 = np.arange(T)[:, None]
    th2 = 2 * np.pi * (f2 + 0.5) * n2 / (2 * T)
    inv = np.concatenate([np.cos(th2), -np.sin(th2)], axis=0) / T
    return jnp.asarray(fwd, bf16), jnp.asarray(inv, bf16)


class _Conv:
    def __init__(self, r0, coef, qT_v, kT_v, vT_v, sk_v, fwd_v, inv_v, aT_v):
        self.rows = pl.ds(pl.multiple_of(r0, 8), 8)
        self.coef = coef
        self.refs = (qT_v, kT_v, vT_v, sk_v, None, fwd_v, inv_v, aT_v)

    def fwd(self):
        _, kT_v, vT_v, sk_v, _, fwd_v, _, _ = self.refs
        rows = self.rows
        k = kT_v[rows, :].astype(f32)
        lane = lax.broadcasted_iota(jnp.int32, (8, S), 1)
        ks = k * self.coef(rows, 0)
        for j in range(1, 4):
            kj = jnp.where(lane >= j, pltpu.roll(k, j, axis=1), 0.0)
            ks = ks + kj * self.coef(rows, j)
        u = ks * vT_v[rows, :].astype(f32)
        self.ud = u * self.coef(rows, 4)
        lhs = jnp.concatenate(_tiles(u) + _tiles(sk_v[rows, :].astype(f32)), axis=0)
        self.x = jnp.dot(lhs.astype(bf16), fwd_v[0:T, :], preferred_element_type=f32)

    def inv(self):
        inv_v = self.refs[6]
        blk = [self.x[r * 8:(r + 1) * 8, :] for r in range(2 * NB)]
        ur = [b[:, :T] for b in blk[:NB]]
        ui = [b[:, T:] for b in blk[:NB]]
        kr = [b[:, :T] for b in blk[NB:]]
        ki = [b[:, T:] for b in blk[NB:]]
        flane = lax.broadcasted_iota(jnp.int32, (8, T), 1)
        sgn = jnp.where((flane & 1) == 0, 1.0, -1.0).astype(f32)
        wr = [sgn * ki[0]] + [kr[a - 1] + sgn * ki[a] for a in range(1, NB)]
        wi = [-(sgn * kr[0])] + [ki[a - 1] - sgn * kr[a] for a in range(1, NB)]
        ys = []
        for a in range(NB):
            yr = wr[0] * ur[a] - wi[0] * ui[a]
            yi = wr[0] * ui[a] + wi[0] * ur[a]
            for dl in range(1, a + 1):
                yr = yr + (wr[dl] * ur[a - dl] - wi[dl] * ui[a - dl])
                yi = yi + (wr[dl] * ui[a - dl] + wi[dl] * ur[a - dl])
            ys.append(jnp.concatenate([yr, yi], axis=1))
        yf = jnp.concatenate(ys, axis=0)
        y = jnp.dot(yf.astype(bf16), inv_v[...], preferred_element_type=f32)
        self.y = jnp.concatenate([y[a * 8:(a + 1) * 8, :] for a in range(NB)], axis=1)

    def gate(self):
        qT_v, aT_v = self.refs[0], self.refs[7]
        out = qT_v[self.rows, :].astype(f32) * (self.y + self.ud)
        aT_v[self.rows, :] = out
        return pltpu.bitcast(out, u32)


class _QBlock:
    def __init__(self, h, i, q_v, k_s, v_s, ctx_v):
        self.h, self.i = h, i
        self.q_v, self.k_s, self.v_s, self.ctx_v = q_v, k_s, v_s, ctx_v
        self.lo = i * QB
        self.end = self.lo + QB
        self.t = []

    def scores(self):
        q = _up(_opq(_pk(self.q_v[self.h, self.lo:self.end, :]), self.h))
        for a in range(0, self.end, KCH):
            b = min(a + KCH, self.end)
            s = lax.dot_general(q, _up(self.k_s[a // 2:b // 2, :]), NT, preferred_element_type=f32)
            self.t += _tiles(s)
        row = lax.broadcasted_iota(jnp.int32, (QB, QB), 0)
        col = lax.broadcasted_iota(jnp.int32, (QB, QB), 1)
        self.t[-1] = jnp.where(col <= row, self.t[-1], NEG)

    def values(self):
        m = jnp.max(_fold(jnp.maximum, self.t), axis=1, keepdims=True)
        if self.i >= 8:
            R = 32
            mb = jnp.broadcast_to(m, (QB, 128))
            ls = []
            for g in range(QB // R):
                mg = mb[g * R:(g + 1) * R]
                if ls:
                    mg = mg + pltpu.bitcast(pltpu.bitcast(ls[-1], u32) & _zero(self.h), f32)
                ls.append(_fold(jnp.add, [jnp.exp2(t[g * R:(g + 1) * R] - mg) for t in self.t]))
            l = jnp.concatenate(ls, axis=0)
        else:
            l = _fold(jnp.add, [jnp.exp2(t - m) for t in self.t])
        off = m + jnp.log2(jnp.sum(l, axis=1, keepdims=True))
        acc = None
        for a in range(0, self.end, KCH):
            b = min(a + KCH, self.end)
            p = jnp.concatenate([jnp.exp2(t - off) for t in self.t[a // 128:b // 128]], axis=1)
            r = jnp.dot(p.astype(bf16), _up(self.v_s[a // 2:b // 2, :]), preferred_element_type=f32)
            acc = r if acc is None else acc + r
        self.ctx_v[self.h, self.lo // 2:self.end // 2, :] = _pk(acc.astype(bf16))


def _head_body(h, c_p, qw_v, k_s, v_s, ctx_v, convs):
    n = S // PB
    w = {}

    def proj(j, half):
        if half not in w:
            w[half] = _up(_opq(_pk(qw_v[H + h, half * C:(half + 1) * C, :]), h))
        rows = slice(j * PB // 2, (j + 1) * PB // 2)
        r = jnp.dot(_up(c_p[rows, :]), w[half], preferred_element_type=f32)
        (k_s, v_s)[half][rows, :] = _pk(r.astype(bf16))

    blk = [_QBlock(h, i, qw_v, k_s, v_s, ctx_v) for i in range(S // QB)]
    c0, c1, c2 = convs
    extra = {(0, 5): c2.inv, (1, 5): c2.gate, (3, 2): c1.fwd, (4, 2): c1.inv, (5, 2): c1.gate,
             (5, 0): c0.fwd, (6, 0): c0.inv, (6, 5): c0.gate}
    proj(0, 0)
    c2.fwd()
    proj(1, 0)
    blk[0].scores()
    blk[1].scores()
    proj(0, 1)
    for j in range(n):
        more = j + 1 < n
        step = [blk[2 * j + 2].scores if more else None,
                (lambda: proj(j + 1, 1)) if more else None,
                blk[2 * j].values,
                blk[2 * j + 3].scores if more else None,
                (lambda: proj(j + 2, 0)) if j + 2 < n else None,
                blk[2 * j + 1].values]
        for p, f in enumerate(step):
            if (j, p) in extra:
                extra[j, p]()
            if f is not None:
                f()


def _kernel(qT_h, kT_h, vT_h, shk_h, sk_h, d_h, xT_h, c_h, wq_h, wuk_h, wuv_h, woT_h,
            fwd_h, inv_h, out_h,
            qT_v, kT_v, vT_v, sk_v, xT_v, x_v, c_v, c_p, wq0_raw, wq1_raw, wq0_p, wq1_p,
            wuk_raw, wuv_raw, qw_v, ctx_v, wo_v, aT_v, coef_v, cw_v, k_s, v_s, o_s, bT_s,
            shk_v, d_v, fwd_v, inv_v,
            sem, sem_x, sem_q0, sem_q1, sem_w, sem_o):
    cp = pltpu.make_async_copy

    a_in = ((kT_h, kT_v), (vT_h, vT_v), (sk_h, sk_v), (qT_h, qT_v))
    a_late = [cp(s.at[0:H * CH], d.at[0:H * CH], sem.at[i]) for i, (s, d) in enumerate(a_in)]
    a_early = [cp(s.at[H * CH:M], d.at[H * CH:M], sem.at[4 + i]) for i, (s, d) in enumerate(a_in)]
    tiny = [cp(shk_h, shk_v, sem.at[8]), cp(d_h, d_v, sem.at[9]), cp(fwd_h, fwd_v, sem.at[10]),
            cp(inv_h, inv_v, sem.at[11])]
    c_copy = cp(c_h, c_v, sem.at[12])
    wo_copy = cp(woT_h, wo_v, sem.at[13])

    def x_copy(j):
        return cp(xT_h.at[:, _rows(j, XR)], xT_v.at[:, _rows(j, XR)], sem_x.at[j])

    def wq0_copy(e, j):
        return cp(wq_h.at[_rows(j, QR), 0:HH, e * 128:(e + 1) * 128], wq0_raw.at[e, _rows(j, QR)],
                  sem_q0.at[e, j])

    def wq1_copy(j):
        return cp(wq_h.at[_rows(j, QR), HH:H, :], wq1_raw.at[_rows(j, QR)], sem_q1.at[j])

    def w_copies(j):
        return (cp(wuk_h.at[_rows(j, WR)], wuk_raw.at[_rows(j, WR)], sem_w.at[0, j]),
                cp(wuv_h.at[_rows(j, WR)], wuv_raw.at[_rows(j, WR)], sem_w.at[1, j]))

    def start_seq(fn, lo, hi):
        def body(j, carry):
            for c in fn(j):
                c.start()
            return carry
        lax.fori_loop(lo, hi, body, 0)

    x_copy(0).start()
    start_seq(lambda j: (wq0_copy(0, j),), 0, NQ)
    for c in tiny:
        c.start()
    start_seq(lambda j: (wq0_copy(1, j),), 0, NQ)
    start_seq(lambda j: (x_copy(j),), 1, NR)
    for c in a_early:
        c.start()
    start_seq(lambda j: (wq1_copy(j),), 0, NQ)
    c_copy.start()
    start_seq(w_copies, 0, NR)
    for c in a_late:
        c.start()
    wo_copy.start()

    def conv(r0, coef):
        return _Conv(r0, coef, qT_v, kT_v, vT_v, sk_v, fwd_v, inv_v, aT_v)

    def coef_col(rows, j):
        return coef_v[rows, :][:, j:j + 1]

    def coef_wide(rows, j):
        return jnp.concatenate([cw_v[j, rows, :]] * NB, axis=1)

    def widen_piece(r):
        def run():
            rows = _rows(r, H * CH // NA)
            col = coef_v[rows, :]
            val = jnp.stack([jnp.broadcast_to(col[:, j:j + 1], (H * CH // NA, 128)) for j in range(5)])
            cw_v[:, rows, :] = val
            return pltpu.bitcast(val, u32)
        return run

    def coef_piece():
        tab = jnp.concatenate([shk_v[...].astype(f32), d_v[...].astype(f32).reshape(1, M),
                               jnp.zeros((3, M), f32)], axis=0)
        coef_v[...] = tab.T

    def xpose_piece(t):
        def run():
            val = _pk(xT_v[:, t * 128:(t + 1) * 128].T)
            x_v[t * 64:(t + 1) * 64, :] = val
            return val[:, 0:MA]
        return run

    def wq0_piece(e, t):
        def run():
            val = _pk(pltpu.einshape("chd->hcd", wq0_raw[e, t * RP:(t + 1) * RP]))
            wq0_p[:, t * (RP // 2):(t + 1) * (RP // 2), e * 128:(e + 1) * 128] = val
            return val
        return run

    def wq1_piece(t):
        def run():
            val = _pk(pltpu.einshape("chd->hcd", wq1_raw[_rows(t, RP)]))
            wq1_p[:, _rows(t, RP // 2), :] = val
            return val
        return run

    def qproj(xs, r0, g, slots, wq_p, pieces, z, span=None):
        span = span or len(slots) - 1
        done = 0
        deps = []
        for k, (hh, s, e) in enumerate(slots):
            cols = slice(None) if e is None else slice(e * 128, (e + 1) * 128)
            qh = jnp.dot(xs[s], _up(wq_p[hh, :, cols]), preferred_element_type=f32)
            if deps:
                vregs = [d[..., t * 8:(t + 1) * 8, u * 128:(u + 1) * 128].reshape(-1, 8, 128)[v]
                         for d in deps for t in range(d.shape[-2] // 8)
                         for u in range(d.shape[-1] // 128)
                         for v in range(d.size // (d.shape[-1] * d.shape[-2]))]
                top = qh[0:8, 0:128] + pltpu.bitcast(_fold(jnp.bitwise_or, vregs) & z, f32)
                if qh.shape[1] > 128:
                    top = jnp.concatenate([top, qh[0:8, 128:]], axis=1)
                qh = jnp.concatenate([top, qh[8:]], axis=0)
                deps = []
            n = xs[s].shape[0]
            o = r0 + s * n
            dst = pl.ds(o, n) if isinstance(o, int) else pl.ds(pl.multiple_of(o, 64), n)
            qw_v[g * HH + hh, dst, cols] = (qh * QSCALE).astype(bf16)
            while done < min(len(pieces), -(-(k + 1) * len(pieces) // span)):
                d = pieces[done]()
                if d is not None:
                    deps.append(d)
                done += 1

    def xs0():
        return [_up(x_v[s * (AR // 2):(s + 1) * (AR // 2), :]) for s in range(XR // AR)]

    bT_s[...] = jnp.zeros(bT_s.shape, f32)
    x_copy(0).wait()
    for t in range(XR // 128):
        xpose_piece(t)()
    for j in range(NQ):
        wq0_copy(0, j).wait()
        for t in range(QR // RP):
            wq0_piece(0, j * (QR // RP) + t)()
    slots = [(hh, s, e) for e in range(2) for hh in range(HH) for s in range(XR // AR)]
    n1, n2 = 7, len(slots) // 2 + 3
    qproj(xs0(), 0, 0, slots[:n1], wq0_p, [], None)
    for c in tiny:
        c.wait()
    for j in range(NQ):
        wq0_copy(1, j).wait()
    zero = _pk(fwd_v[T:T + 16, 0:128])
    qproj(xs0(), 0, 0, slots[n1:n2], wq0_p, [wq0_piece(1, t) for t in range(M // RP)], zero,
          span=len(slots) // 2 - n1 - 1)
    for j in range(1, NR):
        x_copy(j).wait()
    qproj(xs0(), 0, 0, slots[n2:], wq0_p,
          [coef_piece] + [xpose_piece(t) for t in range(XR // 128, S // 128)], zero)
    for c in a_early:
        c.wait()

    def step_a(r, carry):
        @pl.when(r < NQ)
        def _():
            wq1_copy(r).wait()
        x = _up(_opq(x_v[pl.ds(pl.multiple_of(XR // 2 + r * (A1 // 2), 32), A1 // 2), :], r))
        w = [wq1_piece(jnp.minimum(r, NQ - 1) * (QR // RP) + t) for t in range(QR // RP)]
        cv = conv(H * CH + r * 8, coef_col)
        qproj([x], XR + r * A1, 0, [(hh, 0, None) for hh in range(HH)], wq0_p,
              [cv.fwd] + w[:3] + [cv.inv, w[3], cv.gate, widen_piece(r)], _zero(r),
              span=HH - 1)
        return carry
    lax.fori_loop(0, NA, step_a, 0)

    c_copy.wait()

    def step_b(r, carry):
        for c in w_copies(r):
            c.wait()

        def piece(t, w):
            def run():
                src = pl.ds(pl.multiple_of(r * WR + t * RP, RP), RP)
                dst = pl.ds(pl.multiple_of(w * C + r * WR + t * RP, RP), RP)
                qw_v[H:2 * H, dst, :] = pltpu.einshape("chd->hcd", (wuk_raw, wuv_raw)[w][src])
                if w == 0 and t % 2 == 0:
                    k = r * (XR // 64) + t // 2
                    val = _pk(c_v[_rows(k, 64), :])
                    c_p[_rows(k, 32), :] = val
                    return val
            return run
        xs = [_up(_opq(x_v[_rows(r * (XR // AR) + u, AR // 2), :], r)) for u in range(XR // AR)]
        qproj(xs, r * XR, 1, [(hh, u, None) for hh in range(HH) for u in range(XR // AR)], wq1_p,
              [piece(t, w) for t in range(WR // RP) for w in range(2)], _zero(r))
        return carry
    lax.fori_loop(0, NR, step_b, 0)

    for c in a_late:
        c.wait()

    def head(h, carry):
        _head_body(h, c_p, qw_v, k_s, v_s, ctx_v,
                   [conv(h * CH + g * 8, coef_wide) for g in range(CH // 8)])
        return carry
    lax.fori_loop(0, H, head, 0)

    wo_copy.wait()
    no = S // PB

    def emit_a(k):
        val = aT_v[0:MA, _rows(k, PB)].T
        o_s[_rows(k, PB), 0:MA] = val.astype(bf16)
        return _fold(jnp.maximum, _tiles(val))

    def emit_b(rs, bT):
        val = jnp.concatenate([aT_v[MA:M, rs], bT], axis=0).T
        o_s[rs, MA:2 * M] = val.astype(bf16)
        return _fold(jnp.maximum, _tiles(val))

    def copy_a(k):
        return cp(o_s.at[_rows(k, PB), 0:MA], out_h.at[_rows(k, PB), 0:MA], sem_o.at[0, k])

    def copy_b(rs, k):
        return cp(o_s.at[rs, MA:2 * M], out_h.at[rs, MA:2 * M], sem_o.at[1, k])

    def ostep(j, carry):
        dep_b = emit_b(_rows(jnp.maximum(j * OU - 1, 0), PB), bT_s[...])
        for u in range(OU):
            k = j * OU + u
            dep_a = emit_a(k)
            copy_a(k).start()
            bT = None
            for h in range(H):
                cx = ctx_v[h, _rows(k, PB // 2), :]
                if h in (4, 10):
                    cx = _tie(cx, dep_b if h == 4 else dep_a, j)
                r = lax.dot_general(wo_v[h], _up(cx), NT, preferred_element_type=f32)
                bT = r if bT is None else bT + r
            if u + 1 < OU:
                dep_b = emit_b(_rows(k, PB), bT)
                copy_b(_rows(k, PB), k).start()
        bT_s[...] = bT

        @pl.when(j > 0)
        def _():
            copy_b(_rows(j * OU - 1, PB), j * OU - 1).start()
        return carry
    lax.fori_loop(0, no // OU, ostep, 0)
    last = [pl.ds(S - PB + u * 128, 128) for u in range(2)]
    for u in range(2):
        emit_b(last[u], bT_s[:, u * 128:(u + 1) * 128])
        copy_b(last[u], no - 1 + u).start()
    for k in range(no):
        copy_a(k).wait()
    for k in range(no - 1):
        copy_b(_rows(k, PB), k).wait()
    for u in range(2):
        copy_b(last[u], no - 1 + u).wait()


@jax.jit
def pallas_concat_heads__ssm_conv_h3__compressed_kv_cla__prompt_kernel(
    A_q: jax.Array,
    A_k: jax.Array,
    A_v: jax.Array,
    A_shift_k: jax.Array,
    A_ssm_k: jax.Array,
    A_ssm_D: jax.Array,
    B_x: jax.Array,
    B_c_kv: jax.Array,
    B_w_q: jax.Array,
    B_w_uk: jax.Array,
    B_w_uv: jax.Array,
    B_w_o: jax.Array,
):
    fwd, inv = _dft_mats()
    hbm = pl.BlockSpec(memory_space=pltpu.HBM)
    V = pltpu.VMEM
    dma = pltpu.SemaphoreType.DMA
    out = pl.pallas_call(
        _kernel,
        out_shape=jax.ShapeDtypeStruct((S, 2 * M), bf16),
        in_specs=[hbm] * 14,
        out_specs=hbm,
        scratch_shapes=[
            V((M, S), bf16), V((M, S), bf16), V((M, S), bf16), V((M, S), bf16),
            V((M, S), bf16), V((S // 2, M), u32),
            V((S, C), bf16), V((S // 2, C), u32),
            V((2, M, HH, 128), bf16), V((M, HH, D), bf16),
            V((HH, M // 2, D), u32), V((HH, M // 2, D), u32),
            V((C, H, D), bf16), V((C, H, D), bf16),
            V((2 * H, S, D), bf16), V((H, S // 2, D), u32),
            V((H, M, D), bf16), V((M, S), f32), V((M, 8), f32),
            V((5, H * CH, 128), f32),
            V((S // 2, D), u32), V((S // 2, D), u32),
            V((S, 2 * M), bf16), V((M, PB), f32),
            V((4, M), bf16), V((M,), bf16), V((T + 16, 2 * T), bf16), V((2 * T, T), bf16),
            dma((14,)), dma((NR,)), dma((2, NQ)), dma((NQ,)), dma((2, NR)), dma((2, S // PB + 1)),
        ],
        compiler_params=pltpu.CompilerParams(
            vmem_limit_bytes=120 * 1024 * 1024,
            disable_semaphore_checks=True, disable_bounds_checks=True),
    )(A_q[0].T, A_k[0].T, A_v[0].T, A_shift_k.T, A_ssm_k, A_ssm_D, B_x[0].T, B_c_kv[0],
      B_w_q, B_w_uk, B_w_uv, jnp.swapaxes(B_w_o, 1, 2), fwd, inv)
    return out[None]
```
